```python
import os as _os
_os.environ.setdefault("JAX_PLATFORMS", "cpu")
import jax
import jax.numpy as jnp

def _softmax(x, axis=-1):
    return jax.nn.softmax(x, axis=axis)
def _gelu(x):
    return jax.nn.gelu(x, approximate=True)
def _silu(x):
    return jax.nn.silu(x)
def _sigmoid(x):
    return jax.nn.sigmoid(x)
def _layernorm(x, axis=-1, eps=1e-5):
    m = jnp.mean(x, axis=axis, keepdims=True)
    v = jnp.var(x, axis=axis, keepdims=True)
    return (x - m) / jnp.sqrt(v + eps)
def _scatter_add(tgt, idx, src, axis=0):
    return tgt.at[idx].add(src)
def _segment_sum(src, seg, n):
    return jax.ops.segment_sum(src, seg, n)
class _Rng:
    def __init__(self, key):
        self._k = key
    def _next(self):
        self._k, sub = jax.random.split(self._k)
        return sub
    def normal(self, shape):
        return jax.random.normal(self._next(), shape, dtype=jnp.bfloat16)
    def randint(self, lo, hi, shape):
        return jax.random.randint(self._next(), shape, lo, hi, dtype=jnp.int32)
    def uniform(self, shape, lo=0.0, hi=1.0):
        return jax.random.uniform(self._next(), shape, jnp.bfloat16, lo, hi)
    def permutation(self, n):
        return jax.random.permutation(self._next(), n)


kernel_name = 'standalone__layernorm_linear__sampling'

def setup_inputs():
    _rng = _Rng(jax.random.key(int.from_bytes(__import__("os").urandom(4), "little")))
    _w = (lambda a: (lambda t: t.astype(jnp.bfloat16) if jnp.issubdtype(t.dtype, jnp.floating) else t)(jnp.asarray(a)))
    B, S, D = 1024, 32, 576
    return {
        "x": _w((lambda *s: _rng.normal(s) * 0.05)(B, S, D)),
        "g": _w((lambda *s: _rng.normal(s) * 0.05)(D) + 1.0),
        "b": _w((lambda *s: _rng.normal(s) * 0.05)(D)),
        "w": _w((lambda *s: _rng.normal(s) * 0.05)(D, D)),
    }

def reference(x, g, b, w):
    return (_layernorm(x, axis=-1) * g + b) @ w
```

```python
import functools
import numpy as np
import jax, jax.numpy as jnp
from jax import lax
import jax.experimental.pallas as pl
import jax.experimental.pallas.tpu as pltpu
f32=jnp.float32; bf16=jnp.bfloat16; u32=jnp.uint32
S=32; D=576; B=1024; H=288; KH=256; KR=80
def pk(v): return pltpu.bitcast(v, u32)
def up(v): return pltpu.bitcast(v, bf16)
def pk2(a, b): return pltpu.pack_elementwise([a, b], packed_dtype=bf16)
def dot(a,b): return jnp.dot(a,b,preferred_element_type=f32)

def prep_body(w_ref, g_ref, b_ref, as_ref, ar_ref):
    g_row = g_ref[...].astype(f32).reshape(1, D)
    b_row = b_ref[...].astype(f32).reshape(1, D)
    w = w_ref[...]
    rid = lax.broadcasted_iota(jnp.int32, (16, D), 0)
    bmat = jnp.where(rid < 2, jnp.broadcast_to(b_row, (16, D)), 0.0).astype(bf16)
    bias = dot(bmat, w)
    hi = bias.astype(bf16).astype(f32)
    extra = jnp.where(rid == 0, hi, bias - hi)
    def permute_rows(v):
        n = v.shape[0]
        return jnp.concatenate([up(pk2(v[16*q:16*q+8], v[16*q+8:16*q+16])).astype(f32) for q in range(n // 16)], axis=0)
    gpad = jnp.concatenate([g_row, jnp.zeros((1, 64), f32)], axis=1)
    gcol = permute_rows(jnp.broadcast_to(gpad, (128, 640)).T[:D])
    wp = permute_rows(w.astype(f32))
    wpad = jnp.concatenate([wp, jnp.zeros((D, 64), f32)], axis=1)
    wg = wpad * jnp.concatenate([gcol]*5, axis=1)
    xpad = jnp.concatenate([extra, jnp.zeros((16, 64), f32)], axis=1)
    waug = jnp.concatenate([wg, xpad, jnp.zeros((48, 640), f32)], axis=0)
    a = waug.T
    A11=a[:H,:KH];A12=a[:H,KH:2*KH];A21=a[H:D,:KH];A22=a[H:D,KH:2*KH]
    for i, v in enumerate([A11+A22,A21+A22,A11,A22,A11+A12,A21-A11,A12-A22]):
        as_ref[i] = pk(v.astype(bf16))
    ar_ref[...] = pk(a[:D, 2*KH:].astype(bf16))

def make(SPB=1, LA=2, wrap=True, nord=False, nowr=False, nacc=2, explicit=True, quota=176, kr=80, checks=True):
    G = 4 * SPB
    NI = S // SPB

    def kern(x_hbm, w_hbm, g_ref, b_ref, o_hbm, xbuf, obuf, wbuf, as_ref, ar_ref, bs, br, tb, isem, osem, wsem):
        def rd(s):
            return pltpu.make_async_copy(x_hbm.at[s], xbuf.at[s], isem.at[s])
        def wr(s):
            return pltpu.make_async_copy(obuf.at[s], o_hbm.at[s], osem.at[s])
        wcp = pltpu.make_async_copy(w_hbm, wbuf, wsem)
        wcp.start()
        rd(0).start()
        rid = lax.broadcasted_iota(jnp.int32,(kr - 64,128),0)
        ones=(rid<2).astype(f32).astype(bf16)
        for t in range(8): br[t, 32:kr//2, :] = pk(ones)
        wcp.wait()
        for s in range(1, 1 if nord else S): rd(s).start()
        prep_body(wbuf, g_ref, b_ref, as_ref, ar_ref)

        def ln_g(s, g):
            c0 = 256*g
            cols = slice(c0, c0+256)
            ld = lambda r0: xbuf[s, r0:r0+8, cols].astype(f32)
            def tree(accs):
                while len(accs) > 1:
                    accs = [accs[i] + accs[i+1] for i in range(0, len(accs), 2)]
                return accs[0]
            accs = [None]*nacc
            for q in range(D // 8):
                v = ld(8*q)
                accs[q % nacc] = v if accs[q % nacc] is None else accs[q % nacc] + v
                yield 4
            m = jnp.sum(tree(accs), axis=0, keepdims=True) * (1.0 / D)
            m = jnp.broadcast_to(m, (8, 256))
            accs = [None]*nacc
            for q in range(D // 8):
                v = ld(8*q) - m
                v = v * v
                accs[q % nacc] = v if accs[q % nacc] is None else accs[q % nacc] + v
                yield 8
            var = jnp.sum(tree(accs), axis=0, keepdims=True) * (1.0 / D)
            r = jnp.broadcast_to(lax.rsqrt(var + 1e-5), (8, 256))
            def nrm(r0):
                return (ld(r0) - m) * r
            for q in range(KH // 16):
                Bab = []
                for h in range(2):
                    x1 = nrm(16*q + 8*h); x2 = nrm(KH + 16*q + 8*h)
                    B11=x1[:,:128];B12=x1[:,128:];B21=x2[:,:128];B22=x2[:,128:]
                    Bab.append([B11+B22,B11,B12-B22,B21-B11,B22,B11+B12,B21+B22])
                for i in range(7):
                    bs[g, i, q*8:(q+1)*8, :] = pk2(Bab[0][i], Bab[1][i])
                yield 41
            for q in range(4):
                pr = pk2(nrm(2*KH+16*q), nrm(2*KH+16*q+8))
                br[2*g, 8*q:8*q+8, :] = pr[:, :128]
                br[2*g+1, 8*q:8*q+8, :] = pr[:, 128:]
                yield 14

        def mm_g(s, g, tick):
            c0 = 256*g
            Pd = lambda i: dot(up(as_ref[i-1]), up(bs[g, i-1]))
            R = lambda n, mth: dot(up(ar_ref[n*H//2:(n+1)*H//2, :kr]), up(br[2*g+mth]))
            par = g % 2
            vals = {}
            def st(k, v):
                if explicit: tb[par, k] = v
                else: vals[k] = v
            def ldt(k):
                if explicit: return jnp.concatenate([tb[par, k, :144], tb[par, k, 144:]], axis=0)
                return vals[k]
            if g % 2 == 0:
                P5=Pd(5); tick(); P3=Pd(3)
                st(1,P5+P3); st(0,P5); st(3,P3); tick()
                P1=Pd(1); tick(); P7=Pd(7)
                st(0,(P1+P7)-ldt(0))
                st(3,ldt(3)+P1); tick()
                P4=Pd(4); tick(); R11=R(0,0); R12=R(0,1)
                C11=ldt(0)+(P4+R11); C12=ldt(1)+R12
                obuf[s,:H,c0:c0+256]=jnp.concatenate([C11,C12],axis=1).astype(bf16)
                st(2,P4); tick()
                P2=Pd(2); tick(); P6=Pd(6)
                st(2,ldt(2)+P2)
                st(3,ldt(3)+(P6-P2)); tick()
                R21=R(1,0); R22=R(1,1)
                C21=ldt(2)+R21; C22=ldt(3)+R22
                obuf[s,H:,c0:c0+256]=jnp.concatenate([C21,C22],axis=1).astype(bf16)
                tick()
            else:
                P5=Pd(5)
                st(1,P5); tick()
                P3=Pd(3); tick(); P1=Pd(1)
                p5 = ldt(1)
                st(0,P1-p5); st(1,p5+P3); st(3,P3+P1); tick()
                P7=Pd(7); tick(); P4=Pd(4)
                st(0,ldt(0)+(P7+P4)); st(2,P4); tick()
                R11=R(0,0); R12=R(0,1); tick(); P2=Pd(2)
                C11=ldt(0)+R11; C12=ldt(1)+R12
                obuf[s,:H,c0:c0+256]=jnp.concatenate([C11,C12],axis=1).astype(bf16)
                st(2,ldt(2)+P2); st(3,ldt(3)-P2); tick()
                P6=Pd(6); tick(); R21=R(1,0); R22=R(1,1)
                C21=ldt(2)+R21; C22=ldt(3)+(P6+R22)
                obuf[s,H:,c0:c0+256]=jnp.concatenate([C21,C22],axis=1).astype(bf16)
                tick()

        rd(0).wait()
        for g in range(LA):
            for _ in ln_g(0, g): pass

        def phase(j):
            s0 = j * SPB
            def allln():
                for gg in range(LA, G + LA):
                    sl = s0 + gg // 4
                    if gg // 4 == SPB: sl = jnp.minimum(sl, S - 1)
                    yield from ln_g(sl, gg % 4)
            gen = allln()
            state = dict(debt=0)
            def tick(n=quota):
                state['debt'] += n
                while state['debt'] > 0:
                    try: state['debt'] -= next(gen)
                    except StopIteration: return
            for gg in range(G):
                mm_g(s0 + gg // 4, gg % 4, tick)
                if gg % 4 == 3 and not nowr: wr(s0 + gg // 4).start()
            for _ in gen: pass

        def body(j, carry):
            if not nord:
                for k in range(1, SPB + 1):
                    if k < SPB:
                        rd(j * SPB + k).wait()
                    else:
                        @pl.when(j < NI - 1)
                        def _(): rd(j * SPB + k).wait()
            if wrap:
                @pl.when(j >= 0)
                def _(): phase(j)
            else:
                phase(j)
            return carry
        lax.fori_loop(0, NI, body, 0)
        for s in range(0 if nowr else S):
            wr(s).wait()

    def f(x, g, b, w):
        xt = jnp.transpose(x, (1, 2, 0))
        out = pl.pallas_call(
            kern,
            in_specs=[pl.BlockSpec(memory_space=pl.ANY), pl.BlockSpec(memory_space=pl.ANY),
                      pl.BlockSpec(memory_space=pltpu.VMEM),
                      pl.BlockSpec(memory_space=pltpu.VMEM)],
            out_specs=pl.BlockSpec(memory_space=pl.ANY),
            out_shape=jax.ShapeDtypeStruct((S, D, B), x.dtype),
            scratch_shapes=[pltpu.VMEM((S, D, B), bf16), pltpu.VMEM((S, D, B), bf16), pltpu.VMEM((D, D), bf16),
                            pltpu.VMEM((7, H//2, KH), u32), pltpu.VMEM((D//2, 128), u32),
                            pltpu.VMEM((4, 7, KH//2, 128), u32),
                            pltpu.VMEM((8, kr//2, 128), u32),
                            pltpu.VMEM((2, 4, H, 128), f32),
                            pltpu.SemaphoreType.DMA((S,)), pltpu.SemaphoreType.DMA((S,)), pltpu.SemaphoreType.DMA(())],
            compiler_params=pltpu.CompilerParams(vmem_limit_bytes=110*1024*1024,
                disable_bounds_checks=not checks, disable_semaphore_checks=not checks),
        )(xt, w, g, b)
        return jnp.transpose(out, (2, 0, 1))
    return f


_impl = make(SPB=1)

@jax.jit
def pallas_standalone__layernorm_linear__sampling_kernel(x, g, b, w):
    return _impl(x, g, b, w)
```

```python
import functools
import numpy as np
import jax, jax.numpy as jnp
from jax import lax
import jax.experimental.pallas as pl
import jax.experimental.pallas.tpu as pltpu
f32=jnp.float32; bf16=jnp.bfloat16; u32=jnp.uint32
S=32; D=576; B=1024; H=288; KH=256
LN_STATS = 864; LN_NORM = 712
def pk(v): return pltpu.bitcast(v, u32)
def up(v): return pltpu.bitcast(v, bf16)
def pk2(a, b): return pltpu.pack_elementwise([a, b], packed_dtype=bf16)
def dot(a,b): return jnp.dot(a,b,preferred_element_type=f32)

def prep_body(w_ref, g_ref, b_ref, as_ref, ar_ref):
    g_row = g_ref[...].astype(f32).reshape(1, D)
    b_row = b_ref[...].astype(f32).reshape(1, D)
    w = w_ref[...]
    rid = lax.broadcasted_iota(jnp.int32, (16, D), 0)
    bmat = jnp.where(rid < 2, jnp.broadcast_to(b_row, (16, D)), 0.0).astype(bf16)
    bias = dot(bmat, w)
    hi = bias.astype(bf16).astype(f32)
    extra = jnp.where(rid == 0, hi, bias - hi)
    def permute_rows(v):
        n = v.shape[0]
        return jnp.concatenate([up(pk2(v[16*q:16*q+8], v[16*q+8:16*q+16])).astype(f32) for q in range(n // 16)], axis=0)
    gpad = jnp.concatenate([g_row, jnp.zeros((1, 64), f32)], axis=1)
    gcol = permute_rows(jnp.broadcast_to(gpad, (128, 640)).T[:D])
    wp = permute_rows(w.astype(f32))
    wpad = jnp.concatenate([wp, jnp.zeros((D, 64), f32)], axis=1)
    wg = wpad * jnp.concatenate([gcol]*5, axis=1)
    xpad = jnp.concatenate([extra, jnp.zeros((16, 64), f32)], axis=1)
    waug = jnp.concatenate([wg, xpad, jnp.zeros((48, 640), f32)], axis=0)
    a = waug.T
    A11=a[:H,:KH];A12=a[:H,KH:2*KH];A21=a[H:D,:KH];A22=a[H:D,KH:2*KH]
    for i, v in enumerate([A11+A22,A21+A22,A11,A22,A11+A12,A21-A11,A12-A22]):
        as_ref[i] = pk(v.astype(bf16))
    ar_ref[...] = pk(a[:D, 2*KH:].astype(bf16))


def make(nord=False, nowr=False, nacc=1, kr=80, checks=False, J0=0, MS=2, head=(2,2,4,4,4), sla=True, lead=400, trail=200, lastsplit=(2,1,1), fine=False):
    MG = 4 * MS
    nh = sum(head)
    assert nh % 4 == 0 and (4*S - nh) % MG == 0
    NM = (4*S - nh) // MG - 1
    PM = max(MG, max(head))
    assert sum(lastsplit) == 4

    def kern(x_hbm, w_hbm, g_ref, b_ref, o_hbm, xbuf, obuf, wbuf, as_ref, ar_ref, bs0, bs1, br0, br1, tb, sb, flag, isem, osem, hsem, tsem, wsem):
        BS = (bs0, bs1); BR = (br0, br1)
        def rd(s):
            return pltpu.make_async_copy(x_hbm.at[s], xbuf.at[s], isem.at[s])
        def rdh(k):
            return pltpu.make_async_copy(x_hbm.at[0, :, 512*k:512*k+512], xbuf.at[0, :, 512*k:512*k+512], hsem.at[k])
        def wr(s):
            return pltpu.make_async_copy(obuf.at[s], o_hbm.at[s], osem.at[s])
        def wrp(g0, n, k):
            return pltpu.make_async_copy(obuf.at[S-1, :, 256*g0:256*(g0+n)], o_hbm.at[S-1, :, 256*g0:256*(g0+n)], tsem.at[k])
        wcp = pltpu.make_async_copy(w_hbm, wbuf, wsem)
        wcp.start()
        rdh(0).start()
        flag[0] = 1
        rid = lax.broadcasted_iota(jnp.int32,(kr - 64,128),0)
        ones=(rid<2).astype(f32).astype(bf16)
        for brx in BR:
            for t in range(2*PM): brx[t, 32:kr//2, :] = pk(ones)
        wcp.wait()
        rdh(1).start()
        for s in range(1, 1 if nord else S): rd(s).start()
        prep_body(wbuf, g_ref, b_ref, as_ref, ar_ref)

        def tree(accs):
            while len(accs) > 1:
                accs = [accs[i] + accs[i+1] for i in range(0, len(accs), 2)]
            return accs[0]

        def ln_stats(s, g, out):
            cols = slice(256*g, 256*g+256)
            ld = lambda r0: xbuf[s, r0:r0+8, cols].astype(f32)
            accs = [None]*nacc
            for q in range(D // 8):
                v = ld(8*q)
                accs[q % nacc] = v if accs[q % nacc] is None else accs[q % nacc] + v
                yield 4
            m = jnp.sum(tree(accs), axis=0, keepdims=True) * (1.0 / D)
            m = jnp.broadcast_to(m, (8, 256))
            accs = [None]*nacc
            for q in range(D // 8):
                v = ld(8*q) - m
                v = v * v
                accs[q % nacc] = v if accs[q % nacc] is None else accs[q % nacc] + v
                yield 8
            var = jnp.sum(tree(accs), axis=0, keepdims=True) * (1.0 / D)
            r = jnp.broadcast_to(lax.rsqrt(var + 1e-5), (8, 256))
            out.append((m, r))

        def ln_norm(s, g, mr, bs, br, slot):
            cols = slice(256*g, 256*g+256)
            ld = lambda r0: xbuf[s, r0:r0+8, cols].astype(f32)
            m, r = mr
            def nrm(r0):
                return (ld(r0) - m) * r
            for q in range(KH // 16):
                Bab = []
                for h in range(2):
                    x1 = nrm(16*q + 8*h); x2 = nrm(KH + 16*q + 8*h)
                    B11=x1[:,:128];B12=x1[:,128:];B21=x2[:,:128];B22=x2[:,128:]
                    Bab.append([B11+B22,B11,B12-B22,B21-B11,B22,B11+B12,B21+B22])
                for i in range(7):
                    bs[slot, i, q*8:(q+1)*8, :] = pk2(Bab[0][i], Bab[1][i])
                yield 41
            for q in range(4):
                pr = pk2(nrm(2*KH+16*q), nrm(2*KH+16*q+8))
                br[2*slot, 8*q:8*q+8, :] = pr[:, :128]
                br[2*slot+1, 8*q:8*q+8, :] = pr[:, 128:]
                yield 14

        def merge(a, b):
            da = db = 0
            adone = bdone = False
            while not (adone and bdone):
                if (da * LN_STATS <= db * LN_NORM and not adone) or bdone:
                    try:
                        n = next(a); da += n; yield n
                    except StopIteration: adone = True
                else:
                    try:
                        n = next(b); db += n; yield n
                    except StopIteration: bdone = True

        def ln_stream(groups, par, have_first, nxt):
            st = []
            if not groups: return
            if have_first: st.append((sb[0], sb[1]))
            else: yield from ln_stats(*groups[0], st)
            for i, (s, g) in enumerate(groups):
                a = ln_norm(s, g, st[i], BS[par], BR[par], i)
                if i + 1 < len(groups): b = ln_stats(*groups[i+1], st)
                elif nxt is not None: b = ln_stats(*nxt, st)
                else: b = iter(())
                yield from merge(a, b)
            if nxt is not None:
                sb[0] = st[-1][0]; sb[1] = st[-1][1]

        def mm_g(s, g, par_buf, slot, par, tick):
            bs = BS[par_buf]; br = BR[par_buf]
            c0 = 256*g
            def Pd(i):
                if not fine: return dot(up(as_ref[i-1]), up(bs[slot, i-1]))
                a = dot(up(as_ref[i-1, :, :128]), up(bs[slot, i-1, :64]))
                tick(half=True)
                return a + dot(up(as_ref[i-1, :, 128:]), up(bs[slot, i-1, 64:]))
            R = lambda n, mth: dot(up(ar_ref[n*H//2:(n+1)*H//2, :kr]), up(br[2*slot+mth]))
            def st(k, v): tb[par, k] = v
            def ldt(k): return jnp.concatenate([tb[par, k, :144], tb[par, k, 144:]], axis=0)
            if par == 0:
                P5=Pd(5); tick(); P3=Pd(3)
                st(1,P5+P3); st(0,P5); st(3,P3); tick()
                P1=Pd(1); tick(); P7=Pd(7)
                st(0,(P1+P7)-ldt(0))
                st(3,ldt(3)+P1); tick()
                P4=Pd(4); tick(); R11=R(0,0); R12=R(0,1)
                C11=ldt(0)+(P4+R11); C12=ldt(1)+R12
                obuf[s,:H,c0:c0+256]=jnp.concatenate([C11,C12],axis=1).astype(bf16)
                st(2,P4); tick()
                P2=Pd(2); tick(); P6=Pd(6)
                st(2,ldt(2)+P2)
                st(3,ldt(3)+(P6-P2)); tick()
                R21=R(1,0); R22=R(1,1)
                C21=ldt(2)+R21; C22=ldt(3)+R22
                obuf[s,H:,c0:c0+256]=jnp.concatenate([C21,C22],axis=1).astype(bf16)
                tick()
            else:
                P5=Pd(5)
                st(1,P5); tick()
                P3=Pd(3); tick(); P1=Pd(1)
                p5 = ldt(1)
                st(0,P1-p5); st(1,p5+P3); st(3,P3+P1); tick()
                P7=Pd(7); tick(); P4=Pd(4)
                st(0,ldt(0)+(P7+P4)); st(2,P4); tick()
                R11=R(0,0); R12=R(0,1); tick(); P2=Pd(2)
                C11=ldt(0)+R11; C12=ldt(1)+R12
                obuf[s,:H,c0:c0+256]=jnp.concatenate([C11,C12],axis=1).astype(bf16)
                st(2,ldt(2)+P2); st(3,ldt(3)-P2); tick()
                P6=Pd(6); tick(); R21=R(1,0); R22=R(1,1)
                C21=ldt(2)+R21; C22=ldt(3)+(P6+R22)
                obuf[s,H:,c0:c0+256]=jnp.concatenate([C21,C22],axis=1).astype(bf16)
                tick()

        def phase(mm_groups, rpar, ln_groups, have_first, nxt, after_group):
            gen = ln_stream(ln_groups, 1 - rpar, have_first, nxt)
            nstats = len(ln_groups) - (1 if have_first else 0) + (1 if nxt is not None else 0)
            total = LN_NORM * len(ln_groups) + LN_STATS * nstats
            quota = (total - lead - trail) / (9 * len(mm_groups) - 1)
            state = dict(debt=0)
            def tick(n=None, half=False):
                if fine and n is None:
                    n = quota * (9/16)
                state['debt'] += quota if n is None else n
                while state['debt'] > 0:
                    try: state['debt'] -= next(gen)
                    except StopIteration: return
            if lead: tick(lead)
            for i, (s, g) in enumerate(mm_groups):
                mm_g(s, g, rpar, i, i % 2, tick)
                after_group(i)
            for _ in gen: pass

        gl = lambda a, n: [((a + i) // 4, (a + i) % 4) for i in range(n)]
        waited = set()
        def need(gmax):
            for s in range((gmax + 3) // 4):
                if s == 0:
                    for k in range(2):
                        if 2*k < gmax and ('h', k) not in waited:
                            rdh(k).wait(); waited.add(('h', k))
                elif s not in waited and not nord:
                    rd(s).wait(); waited.add(s)

        ex = 1 if sla else 0
        need(head[0])
        for _ in ln_stream(gl(0, head[0]), 0, False, None): pass
        pos = 0; par = 0
        sizes = list(head) + [MG]
        for k in range(len(head)):
            nxt_pos = pos + sizes[k]
            last = k == len(head) - 1
            exk = ex if last else 0
            need(nxt_pos + sizes[k+1] + exk)
            def hphase(pos=pos, k=k, par=par, nxt_pos=nxt_pos, exk=exk):
                def ag(i):
                    if J0 == 0 and not nowr and (pos + i) % 4 == 3: wr((pos + i) // 4).start()
                phase(gl(pos, sizes[k]), par, gl(nxt_pos, sizes[k+1]), False, gl(nxt_pos + sizes[k+1], 1)[0] if exk else None, ag)
            pl.when(flag[0] == 1)(hphase)
            pos = nxt_pos; par = 1 - par
        s_base = nh // 4
        par0 = par
        already = max([w for w in waited if isinstance(w, int)] + [0])
        def body(k, carry):
            s0 = s_base + k * MS
            if not nord:
                hi = 2*MS + ex
                for rel in range(hi - MS, hi):
                    sk = s0 + rel
                    @pl.when(jnp.logical_and(sk > already, sk < S))
                    def _(): rd(sk).wait()
            if J0 > 0 and not nowr:
                @pl.when(k == J0)
                def _():
                    for s in range(s_base + J0 * MS): wr(s).start()
            mmg = [(s0 + i // 4, i % 4) for i in range(MG)]
            lng = [(jnp.minimum(s0 + MS + i // 4, S - 1), i % 4) for i in range(MG)]
            nx = (jnp.minimum(s0 + 2*MS, S - 1), 0) if sla else None
            def ag(i):
                if nowr: return
                if i % 4 == 3:
                    if J0 > 0:
                        @pl.when(k >= J0)
                        def _(): wr(s0 + i // 4).start()
                    else:
                        wr(s0 + i // 4).start()
            @pl.when(k % 2 == 0)
            def _(): phase(mmg, par0, lng, sla, nx, ag)
            @pl.when(k % 2 == 1)
            def _(): phase(mmg, 1 - par0, lng, sla, nx, ag)
            return carry
        lax.fori_loop(0, NM, body, 0)
        if not nord:
            for s in range(min(S, s_base + (NM - 1) * MS + 2*MS + ex), S): rd(s).wait()
        cuts = {}
        c = 0
        for t, n in enumerate(lastsplit):
            cuts[MG - 4 + c + n - 1] = (c, n, t); c += n
        def agl(i):
            if nowr: return
            if i in cuts: wrp(*cuts[i]).start()
            elif i % 4 == 3: wr(S - MS + i // 4).start()
        phase(gl(4*S - MG, MG), par0 if NM % 2 == 0 else 1 - par0, [], False, None, agl)
        if not nowr:
            for s in range(S - 1): wr(s).wait()
            c = 0
            for t, n in enumerate(lastsplit):
                wrp(c, n, t).wait(); c += n

    def f(x, g, b, w):
        xt = jnp.transpose(x, (1, 2, 0))
        out = pl.pallas_call(
            kern,
            in_specs=[pl.BlockSpec(memory_space=pl.ANY), pl.BlockSpec(memory_space=pl.ANY),
                      pl.BlockSpec(memory_space=pltpu.VMEM),
                      pl.BlockSpec(memory_space=pltpu.VMEM)],
            out_specs=pl.BlockSpec(memory_space=pl.ANY),
            out_shape=jax.ShapeDtypeStruct((S, D, B), x.dtype),
            scratch_shapes=[pltpu.VMEM((S, D, B), bf16), pltpu.VMEM((S, D, B), bf16), pltpu.VMEM((D, D), bf16),
                            pltpu.VMEM((7, H//2, KH), u32), pltpu.VMEM((D//2, 128), u32),
                            pltpu.VMEM((PM, 7, KH//2, 128), u32), pltpu.VMEM((PM, 7, KH//2, 128), u32),
                            pltpu.VMEM((2*PM, kr//2, 128), u32), pltpu.VMEM((2*PM, kr//2, 128), u32),
                            pltpu.VMEM((2, 4, H, 128), f32), pltpu.VMEM((2, 8, 256), f32), pltpu.SMEM((1,), jnp.int32),
                            pltpu.SemaphoreType.DMA((S,)), pltpu.SemaphoreType.DMA((S,)), pltpu.SemaphoreType.DMA((2,)),
                            pltpu.SemaphoreType.DMA((4,)), pltpu.SemaphoreType.DMA(())],
            compiler_params=pltpu.CompilerParams(vmem_limit_bytes=120*1024*1024,
                disable_bounds_checks=not checks, disable_semaphore_checks=not checks),
        )(xt, w, g, b)
        return jnp.transpose(out, (2, 0, 1))
    return f

_impl = make(J0=5)

@jax.jit
def pallas_standalone__layernorm_linear__sampling_kernel(x, g, b, w):
    return _impl(x, g, b, w)
```

```python
import functools
import numpy as np
import jax, jax.numpy as jnp
from jax import lax
import jax.experimental.pallas as pl
import jax.experimental.pallas.tpu as pltpu
f32=jnp.float32; bf16=jnp.bfloat16; u32=jnp.uint32
S=32; D=576; B=1024; KH=256; NT=192; KR=80
def pk(v): return pltpu.bitcast(v, u32)
def up(v): return pltpu.bitcast(v, bf16)
def pk2(a, b): return pltpu.pack_elementwise([a, b], packed_dtype=bf16)
def dot(a,b): return jnp.dot(a,b,preferred_element_type=f32)

def a_operands(A):
    (A11,A12),(A21,A22),(A31,A32) = A
    p2 = A11 - A12; p5 = A21 - A22; p8 = p2 + A31; p13 = p5 - A32
    return [A11+A21, A12+A21, p2, A21, A12+A22, p5, A12, A11+A31, p8, A31, p8-A32, A32, A22+A32, p13, p13+A31]

def b_operands(Bk):
    if len(Bk) == 3:
        (B11,B21),(B12,B22),(B13,B23) = Bk
        s1 = B11+B21; s2 = B12+B22; s3 = B13+B23
        return [B11+B12, B11-B22, B11, s2, B21+B22, B22, s1, s1+s3, s1+B23, B13, B21+B23, B23, s2+s3, s2+B13, B12+B13]
    (B11,B21),(B12,B22) = Bk
    return [B11+B12, B11-B22, B11, B12+B22, B21+B22, B22, B11+B21, B21, B12]
PAIR_SLOT = {0:0, 1:1, 2:2, 3:3, 4:4, 5:5, 6:6, 8:6, 10:7, 13:3, 14:8}

def prep_body(w_ref, g_ref, b_ref, as_ref, ar_ref):
    g_row = g_ref[...].astype(f32).reshape(1, D)
    b_row = b_ref[...].astype(f32).reshape(1, D)
    w = w_ref[...]
    rid = lax.broadcasted_iota(jnp.int32, (16, D), 0)
    bmat = jnp.where(rid < 2, jnp.broadcast_to(b_row, (16, D)), 0.0).astype(bf16)
    bias = dot(bmat, w)
    hi = bias.astype(bf16).astype(f32)
    extra = jnp.where(rid == 0, hi, bias - hi)
    def permute_rows(v):
        n = v.shape[0]
        return jnp.concatenate([up(pk2(v[16*q:16*q+8], v[16*q+8:16*q+16])).astype(f32) for q in range(n // 16)], axis=0)
    gpad = jnp.concatenate([g_row, jnp.zeros((1, 64), f32)], axis=1)
    gcol = permute_rows(jnp.broadcast_to(gpad, (128, 640)).T[:D])
    wp = permute_rows(w.astype(f32))
    wpad = jnp.concatenate([wp, jnp.zeros((D, 64), f32)], axis=1)
    wg = wpad * jnp.concatenate([gcol]*5, axis=1)
    xpad = jnp.concatenate([extra, jnp.zeros((16, 64), f32)], axis=1)
    waug = jnp.concatenate([wg, xpad, jnp.zeros((48, 640), f32)], axis=0)
    a = waug.T
    A = [(a[NT*i:NT*(i+1), :KH], a[NT*i:NT*(i+1), KH:2*KH]) for i in range(3)]
    for i, v in enumerate(a_operands(A)):
        as_ref[i] = pk(v.astype(bf16))
    ar_ref[...] = pk(a[:D, 2*KH:].astype(bf16))

STATS_OPS = 864
def norm_ops(n): return 32 * (75 if n == 3 else 12*2 + 8 + 10 + 9) + n * 4 * 14

def make(nord=False, nowr=False, checks=False, J0=4, lead=400, trail=-300, wts=(1, 1, 1), fuse_prep=False, tailmode=1, NCH=2):
    U = 2
    NTRI = 10
    wL, wQ, wR = wts

    def kern(x_hbm, w_hbm, g_ref, b_ref, o_hbm, xbuf, obuf, wbuf, as_ref, ar_ref, bs0, bs1, br0, br1, tb, sb, flag, isem, osem, tsem, wsem):
        BS = (bs0, bs1); BR = (br0, br1)
        pchunks = [(0, 256), (256, 256), (512, 512)]
        def rdp(i):
            c0, nc = pchunks[i]
            return pltpu.make_async_copy(x_hbm.at[pl.ds(0, 2), :, pl.ds(c0, nc)], xbuf.at[pl.ds(0, 2), :, pl.ds(c0, nc)], isem.at[i])
        def rdt(t, h):
            return pltpu.make_async_copy(x_hbm.at[pl.ds(2 + 3*t, 3), :, pl.ds(512*h, 512)], xbuf.at[pl.ds(2 + 3*t, 3), :, pl.ds(512*h, 512)], isem.at[3 + 2*t + h])
        def wrs(s0, ns, k):
            return pltpu.make_async_copy(obuf.at[pl.ds(s0, ns)], o_hbm.at[pl.ds(s0, ns)], osem.at[k])
        def wrblk(sl, k):
            return pltpu.make_async_copy(obuf.at[sl], o_hbm.at[sl], tsem.at[k])
        wcp = pltpu.make_async_copy(w_hbm, wbuf, wsem)
        def start_rest():
            for i in range(1, 3): rdp(i).start()
            if not nord:
                for t in range(NTRI):
                    for h in range(2): rdt(t, h).start()
        if fuse_prep:
            rdp(0).start(); wcp.start()
        else:
            wcp.start(); rdp(0).start()
        flag[0] = 1
        rid = lax.broadcasted_iota(jnp.int32,(KR - 64, 256),0)
        ones = pk((rid<2).astype(f32).astype(bf16))
        for brx in BR:
            for t in range(U):
                for j in range(3): brx[t, j, 32:KR//2, :] = ones
        if not fuse_prep:
            wcp.wait()
            start_rest()
            prep_body(wbuf, g_ref, b_ref, as_ref, ar_ref)

        def ln_stats(unit, sslot):
            sl, g = unit
            cols = slice(256*g, 256*g+256)
            for j, s in enumerate(sl):
                ld = lambda r0: xbuf[s, r0:r0+8, cols].astype(f32)
                acc = None
                for q in range(D // 8):
                    v = ld(8*q)
                    acc = v if acc is None else acc + v
                    yield 4
                m = jnp.sum(acc, axis=0, keepdims=True) * (1.0 / D)
                m = jnp.broadcast_to(m, (8, 256))
                acc = None
                for q in range(D // 8):
                    v = ld(8*q) - m
                    v = v * v
                    acc = v if acc is None else acc + v
                    yield 8
                var = jnp.sum(acc, axis=0, keepdims=True) * (1.0 / D)
                sb[sslot, j, 0] = m
                sb[sslot, j, 1] = jnp.broadcast_to(lax.rsqrt(var + 1e-5), (8, 256))

        def ln_norm(unit, sslot, par, slot):
            sl, g = unit
            n = len(sl)
            bs = BS[par]; br = BR[par]
            for q in range(KH // 16):
                for t in range(2):
                    lanes = slice(128*t, 128*t+128)
                    cols = slice(256*g + 128*t, 256*g + 128*t + 128)
                    ops = []
                    for h in range(2):
                        Bk = []
                        for j, s in enumerate(sl):
                            m = sb[sslot, j, 0, :, lanes]; r = sb[sslot, j, 1, :, lanes]
                            r0 = 16*q + 8*h
                            Bk.append(((xbuf[s, r0:r0+8, cols].astype(f32) - m) * r,
                                       (xbuf[s, KH+r0:KH+r0+8, cols].astype(f32) - m) * r))
                        ops.append(b_operands(Bk))
                    for i in range(len(ops[0])):
                        bs[slot, i, q*8:(q+1)*8, lanes] = pk2(ops[0][i], ops[1][i])
                    yield 75 if n == 3 else 51
            cols = slice(256*g, 256*g+256)
            for j, s in enumerate(sl):
                m = sb[sslot, j, 0]; r = sb[sslot, j, 1]
                for q in range(4):
                    r0 = 2*KH + 16*q
                    br[slot, j, 8*q:8*q+8, :] = pk2((xbuf[s, r0:r0+8, cols].astype(f32) - m) * r,
                                                    (xbuf[s, r0+8:r0+16, cols].astype(f32) - m) * r)
                    yield 14

        def merge(a, wa, b, wb):
            da = db = 0
            adone = bdone = False
            while not (adone and bdone):
                if (da * wb <= db * wa and not adone) or bdone:
                    try:
                        n = next(a); da += n; yield n
                    except StopIteration: adone = True
                else:
                    try:
                        n = next(b); db += n; yield n
                    except StopIteration: bdone = True


        def ln_stream(units, par, have_first, nxt):
            if not units: return
            ss = [5 if have_first else 0] + list(range(1, len(units)))
            if not have_first: yield from ln_stats(units[0], ss[0])
            for i, u in enumerate(units):
                a = ln_norm(u, ss[i], par, i)
                if i + 1 < len(units): nu, nsl = units[i+1], ss[i+1]
                else: nu, nsl = nxt, 5
                if nu is None: yield from a
                else: yield from merge(a, norm_ops(len(u[0])), ln_stats(nu, nsl), STATS_OPS * len(nu[0]))

        def ln_total(units, have_first, nxt):
            tot = sum(norm_ops(len(u[0])) for u in units)
            st = units[(1 if have_first else 0):] + ([nxt] if nxt is not None else [])
            return tot + sum(STATS_OPS * len(u[0]) for u in st)

        def mm_unit(unit, par, slot, odd, tick, done):
            sl, g = unit
            n = len(sl)
            bs = BS[par]; br = BR[par]
            cols = slice(256*g, 256*g+256)
            tp = slot % 2
            RC = NT // NCH
            def P(k):
                kb = k if n == 3 else PAIR_SLOT[k]
                def f(r):
                    rr = slice(r.start // 2, r.stop // 2)
                    return dot(up(as_ref[k, rr, :]), up(bs[slot, kb]))
                return f
            def REM(i, j):
                def f(r):
                    rr = slice(96*i + r.start // 2, 96*i + r.stop // 2)
                    return dot(up(ar_ref[rr, :KR]), up(br[slot, j]))
                return f
            def rnd(w, post, fins=()):
                for c in range(NCH):
                    r = slice(RC*c, RC*(c+1))
                    def st(k, v): tb[tp, k, r] = v
                    def ld(k): return tb[tp, k, r]
                    def fin(i, j, v): obuf[sl[j], NT*i + RC*c:NT*i + RC*(c+1), cols] = v.astype(bf16)
                    post(r, st, ld, fin)
                    tick(w / NCH)
                for ij in fins: done(*ij)
            D2, D6, D3, D5, D9, D11, R1, R8, R13, Ua, Ub, Uc, Ud, Ue, Uf, X33 = range(16)
            def raw(k, p, w=None): rnd(wL if w is None else w, lambda r, st, ld, fin: st(k, p(r)))
            if n == 3 and odd:
                raw(X33, REM(2, 2), wL / 2)
            raw(D2, P(2)); raw(D6, P(6)); raw(D3, P(3)); raw(D5, P(5))
            a = REM(0, 0); b = REM(1, 1)
            def post(r, st, ld, fin):
                fin(0, 0, a(r) + (ld(D6) + ld(D2))); fin(1, 1, b(r) + (ld(D3) - ld(D5)))
            rnd(wR, post, [(0, 0), (1, 1)])
            raw(R1, P(1))
            a = REM(0, 1); b = REM(1, 0)
            def post(r, st, ld, fin):
                st(Ua, a(r) - (ld(D2) + ld(D3))); st(Ub, b(r) + (ld(D5) - ld(D6)))
            rnd(wR, post)
            p = P(0); rnd(wQ, lambda r, st, ld, fin: fin(0, 1, p(r) + (ld(Ua) - ld(R1))), [(0, 1)])
            p = P(4); rnd(wQ, lambda r, st, ld, fin: fin(1, 0, p(r) + (ld(Ub) + ld(R1))), [(1, 0)])
            if n == 3:
                raw(D9, P(9))
                p = P(11)
                def post(r, st, ld, fin):
                    v = p(r)
                    st(D11, v)
                    if odd: fin(2, 2, v + (ld(D9) + ld(X33)))
                rnd(wQ if odd else wL, post, [(2, 2)] if odd else [])
                a = REM(0, 2); b = REM(2, 0)
                def post(r, st, ld, fin):
                    st(Uc, a(r) - (ld(D6) + ld(D9))); st(Ud, b(r) - (ld(D11) + ld(D2)))
                rnd(wR, post)
                raw(R8, P(8))
                p = P(7); rnd(wQ, lambda r, st, ld, fin: fin(0, 2, p(r) + (ld(Uc) - ld(R8))), [(0, 2)])
                p = P(10); rnd(wQ, lambda r, st, ld, fin: fin(2, 0, (ld(Ud) + ld(R8)) - p(r)), [(2, 0)])
                a = REM(1, 2); b = REM(2, 1)
                def post(r, st, ld, fin):
                    st(Ue, a(r) - (ld(D3) + ld(D11))); st(Uf, b(r) + (ld(D5) - ld(D9)))
                rnd(wR, post)
                raw(R13, P(13))
                p = P(12); rnd(wQ, lambda r, st, ld, fin: fin(1, 2, p(r) + (ld(Ue) + ld(R13))), [(1, 2)])
                p = P(14); rnd(wQ, lambda r, st, ld, fin: fin(2, 1, p(r) + (ld(Uf) - ld(R13))), [(2, 1)])
                if not odd:
                    p = REM(2, 2); rnd(wQ / 2, lambda r, st, ld, fin: fin(2, 2, p(r) + (ld(D9) + ld(D11))), [(2, 2)])
            else:
                a = REM(2, 0); b = REM(2, 1)
                def post(r, st, ld, fin):
                    st(Ud, a(r) - ld(D2)); st(Uf, b(r) + ld(D5))
                rnd(wR, post)
                p = P(8); rnd(wL, lambda r, st, ld, fin: st(R8, p(r) + ld(Ud)))
                p = P(10); rnd(wQ, lambda r, st, ld, fin: fin(2, 0, ld(R8) - p(r)), [(2, 0)])
                p = P(13); rnd(wL, lambda r, st, ld, fin: st(R13, ld(Uf) - p(r)))
                p = P(14); rnd(wQ, lambda r, st, ld, fin: fin(2, 1, p(r) + ld(R13)), [(2, 1)])

        def wsum(n, odd):
            if n == 2: return 7*wL + 3*wR + 4*wQ
            return (9.5*wL - wL + wQ if odd else 9*wL + wQ/2) + 4*wR + 6*wQ

        def phase(mm_units, rpar, ln_units, have_first, nxt, after_unit, done=lambda u, i, j: None):
            gen = ln_stream(ln_units, 1 - rpar, have_first, nxt)
            total = ln_total(ln_units, have_first, nxt) if ln_units else 0
            odds = []; o = False
            for u in mm_units:
                odds.append(o)
                if len(u[0]) == 3: o = not o
            wtot = sum(wsum(len(u[0]), od) for u, od in zip(mm_units, odds))
            quota = max(total - lead - trail, 0) / wtot
            state = dict(debt=0)
            def tick(w=None, n=None):
                state['debt'] += quota * w if n is None else n
                while state['debt'] > 0:
                    try: state['debt'] -= next(gen)
                    except StopIteration: return
            if lead: tick(n=lead)
            for i, u in enumerate(mm_units):
                mm_unit(u, rpar, i, odds[i], tick, functools.partial(done, i))
                after_unit(i)
            for _ in gen: pass

        pu = [([0, 1], g) for g in range(4)]
        tu = lambda s0, g: ([s0, s0 + 1, s0 + 2], g)
        nop = lambda i: None
        rdp(0).wait()
        for _ in ln_stream(pu[0:1], 0, False, None): pass
        if fuse_prep:
            wcp.wait()
            start_rest()
        rdp(1).wait()
        @pl.when(flag[0] == 1)
        def _():
            if fuse_prep: prep_body(wbuf, g_ref, b_ref, as_ref, ar_ref)
            phase(pu[0:1], 0, pu[1:2], False, None, nop)
        rdp(2).wait()
        pl.when(flag[0] == 1)(lambda: phase(pu[1:2], 1, pu[2:4], False, None, nop))
        if not nord:
            rdt(0, 0).wait(); rdt(0, 1).wait()
        pl.when(flag[0] == 1)(lambda: phase(pu[2:4], 0, [tu(2, 0), tu(2, 1)], False, tu(2, 2), nop))
        cl = lambda s: jnp.minimum(s, S - 1)
        tails = []
        def body(t, carry):
            s0 = 2 + 3*t
            sn = [cl(s0 + 3), cl(s0 + 4), cl(s0 + 5)]
            sc = [cl(s0), cl(s0 + 1), cl(s0 + 2)]
            if not nord:
                @pl.when(t < NTRI - 1)
                def _(): rdt(t + 1, 0).wait()
            if not nowr:
                @pl.when(t == J0)
                def _(): wrs(0, 2 + 3*J0, 0).start()
            def auA(i):
                if nowr or i != U - 1: return
                @pl.when(t == NTRI - 1)
                def _(): wrblk((pl.ds(S - 3, 3), slice(None), pl.ds(0, 512)), 0).start()
            pl.when(flag[0] == 1)(lambda: phase([tu(s0, 0), tu(s0, 1)], 1, [(sc, 2), (sc, 3)], True, (sn, 0), auA))
            if not nord:
                @pl.when(t < NTRI - 1)
                def _(): rdt(t + 1, 1).wait()
            @pl.when(t < (NTRI - 1) * flag[0])
            def _():
                def auB(i):
                    if nowr or i != U - 1: return
                    @pl.when(t >= J0)
                    def _(): wrs(s0, 3, 1 + t).start()
                phase([tu(s0, 2), tu(s0, 3)], 0, [(sn, 0), (sn, 1)], True, (sn, 2), auB)
            return carry
        lax.fori_loop(0, NTRI, body, 0)
        def go(sl):
            c = wrblk(sl, 1 + len(tails)); c.start(); tails.append(c)
        def au_last(i):
            if nowr or i == U - 1: return
            go((pl.ds(S - 3, 3), slice(None), pl.ds(512, 256)))
        def done_last(u, i, j):
            if nowr or u != U - 1: return
            cols = pl.ds(768, 256)
            if tailmode == 1:
                go((S - 3 + j, pl.ds(NT*i, NT), cols))
            else:
                if (i, j) == (1, 0): go((pl.ds(S - 3, 2), pl.ds(0, 2*NT), cols))
                if (i, j) == (2, 0):
                    go((S - 3, pl.ds(2*NT, NT), cols)); go((S - 1, pl.ds(0, NT), cols)); go((S - 1, pl.ds(2*NT, NT), cols))
                if (i, j) == (1, 2): go((S - 1, pl.ds(NT, NT), cols))
                if (i, j) == (2, 1): go((S - 2, pl.ds(2*NT, NT), cols))
        phase([tu(S - 3, 2), tu(S - 3, 3)], 0, [], False, None, au_last, done_last)
        if not nowr:
            wrs(0, 2 + 3*J0, 0).wait()
            for t in range(J0, NTRI - 1): wrs(2 + 3*t, 3, 1 + t).wait()
            wrblk((pl.ds(S - 3, 3), slice(None), pl.ds(0, 512)), 0).wait()
            for c in tails: c.wait()

    def f(x, g, b, w):
        xt = jnp.transpose(x, (1, 2, 0))
        out = pl.pallas_call(
            kern,
            in_specs=[pl.BlockSpec(memory_space=pl.ANY), pl.BlockSpec(memory_space=pl.ANY),
                      pl.BlockSpec(memory_space=pltpu.VMEM),
                      pl.BlockSpec(memory_space=pltpu.VMEM)],
            out_specs=pl.BlockSpec(memory_space=pl.ANY),
            out_shape=jax.ShapeDtypeStruct((S, D, B), x.dtype),
            scratch_shapes=[pltpu.VMEM((S, D, B), bf16), pltpu.VMEM((S, D, B), bf16), pltpu.VMEM((D, D), bf16),
                            pltpu.VMEM((15, NT//2, KH), u32), pltpu.VMEM((D//2, 128), u32),
                            pltpu.VMEM((U, 15, KH//2, 256), u32), pltpu.VMEM((U, 15, KH//2, 256), u32),
                            pltpu.VMEM((U, 3, KR//2, 256), u32), pltpu.VMEM((U, 3, KR//2, 256), u32),
                            pltpu.VMEM((2, 16, NT, 256), f32), pltpu.VMEM((6, 3, 2, 8, 256), f32), pltpu.SMEM((1,), jnp.int32),
                            pltpu.SemaphoreType.DMA((3 + 2*NTRI,)), pltpu.SemaphoreType.DMA((NTRI + 1,)),
                            pltpu.SemaphoreType.DMA((12,)), pltpu.SemaphoreType.DMA(())],
            compiler_params=pltpu.CompilerParams(vmem_limit_bytes=120*1024*1024,
                disable_bounds_checks=not checks, disable_semaphore_checks=not checks),
        )(xt, w, g, b)
        return jnp.transpose(out, (2, 0, 1))
    return f

_impl = make()

@jax.jit
def pallas_standalone__layernorm_linear__sampling_kernel(x, g, b, w):
    return _impl(x, g, b, w)
```

```python
import functools, itertools
import numpy as np
import jax, jax.numpy as jnp
from jax import lax
import jax.experimental.pallas as pl
import jax.experimental.pallas.tpu as pltpu
f32=jnp.float32; bf16=jnp.bfloat16; u32=jnp.uint32
S=32; D=576; B=1024; KH=256; NQ=144; KR=80; NQD=8
LAM=(-1.5,-0.5,0.5,1.5)
PAIRS=[(0,1),(0,2),(1,2),(0,3),(1,3),(2,3)]
def pk(v): return pltpu.bitcast(v, u32)
def up(v): return pltpu.bitcast(v, bf16)
def pk2(a, b): return pltpu.pack_elementwise([a, b], packed_dtype=bf16)
def dot(a,b): return jnp.dot(a,b,preferred_element_type=f32)

def a_operands(A1, A2):
    Y = [LAM[i] * A1[i] + A2[i] for i in range(4)]
    out = list(A1) + Y
    for (i, j) in PAIRS:
        d = LAM[j] - LAM[i]
        r = Y[i] + Y[j]
        if d != 1.0: r = r * (1.0 / d)
        out += [r, r + A1[i], A1[j] - r]
    return out

def prep_body(w_ref, g_ref, b_ref, af_ref, as_ref, ar_ref):
    g_row = g_ref[...].astype(f32).reshape(1, D)
    b_row = b_ref[...].astype(f32).reshape(1, D)
    w = w_ref[...]
    rid = lax.broadcasted_iota(jnp.int32, (16, D), 0)
    bmat = jnp.where(rid < 2, jnp.broadcast_to(b_row, (16, D)), 0.0).astype(bf16)
    bias = dot(bmat, w)
    hi = bias.astype(bf16).astype(f32)
    extra = jnp.where(rid == 0, hi, bias - hi)
    def permute_rows(v):
        n = v.shape[0]
        return jnp.concatenate([up(pk2(v[16*q:16*q+8], v[16*q+8:16*q+16])).astype(f32) for q in range(n // 16)], axis=0)
    gpad = jnp.concatenate([g_row, jnp.zeros((1, 64), f32)], axis=1)
    gcol = permute_rows(jnp.broadcast_to(gpad, (128, 640)).T[:D])
    wp = permute_rows(w.astype(f32))
    wpad = jnp.concatenate([wp, jnp.zeros((D, 64), f32)], axis=1)
    wg = wpad * jnp.concatenate([gcol]*5, axis=1)
    xpad = jnp.concatenate([extra, jnp.zeros((16, 64), f32)], axis=1)
    waug = jnp.concatenate([wg, xpad, jnp.zeros((48, 640), f32)], axis=0)
    a = waug.T
    for kt in range(5):
        af_ref[kt] = a[:D, 128*kt:128*(kt+1)]
    for q in range(NQ // 16):
        for kt in range(2):
            ops = []
            for par in range(2):
                A1 = [af_ref[kt, pl.ds(NQ*i + 16*q + par, 8, stride=2), :] for i in range(4)]
                A2 = [af_ref[2 + kt, pl.ds(NQ*i + 16*q + par, 8, stride=2), :] for i in range(4)]
                ops.append(a_operands(A1, A2))
            for k in range(26):
                as_ref[k, 8*q:8*q+8, 128*kt:128*(kt+1)] = pk2(ops[0][k], ops[1][k])
    for q in range(D // 16):
        ar_ref[8*q:8*q+8, :] = pk2(af_ref[4, pl.ds(16*q, 8, stride=2), :], af_ref[4, pl.ds(16*q + 1, 8, stride=2), :])


def b_operands(B1, B2):
    mult = [{} for _ in range(4)]
    def mul(j, c):
        if c == 1.0: return B2[j]
        if c not in mult[j]: mult[j][c] = B2[j] * c
        return mult[j][c]
    E = [B1[i] - mul(i, LAM[i]) if LAM[i] > 0 else B1[i] + mul(i, -LAM[i]) for i in range(4)]
    for i in range(4): yield i, E[i]
    for i in range(4): yield 4 + i, B2[i]
    for p, (i, j) in enumerate(PAIRS):
        d = LAM[j] - LAM[i]
        s = E[i] + E[j]
        yield 8 + 3*p, s
        yield 9 + 3*p, s + mul(j, d)
        yield 10 + 3*p, s - mul(i, d)

N_OPS = 16*3 + 2*32 + 26

def make(nord=False, nowr=False, checks=False, J0=3, lead=100, trail=-100, nacc=1, hnacc=1, pnacc=1, psplit=1, onepass=True, nsub=3, mainop=True, JB=True, tailmode=0, notail=False, nobulk=False, rows=(48, 48, 48), hrows=(48, 48, 48), plan=(1.0, 1.33, 1.33, 1.33, 3.0, 3.0), verbose=False):
    SOPS = 355 if onepass else 432

    def kern(x_hbm, w_hbm, g_hbm, b_hbm, o_hbm, xbuf, obuf, wbuf, g_ref, b_ref, af_ref, as_ref, ar_ref, bs, br, tb, sb, flag, isem, osem, tsem):
        chunks = [(0,0,128), (0,128,128), (0,256,256), (0,512,256), (0,768,256), (4,0,256), (4,256,256), (4,512,512)]
        NC = len(chunks)
        def rdp(i):
            s0, c0, nc = chunks[i]
            sl = (pl.ds(s0, 4), slice(None), pl.ds(c0, nc))
            return pltpu.make_async_copy(x_hbm.at[sl], xbuf.at[sl], isem.at[i])
        def rdq(q):
            return pltpu.make_async_copy(x_hbm.at[pl.ds(4*q, 4)], xbuf.at[pl.ds(4*q, 4)], isem.at[NC + q])
        def wrs(s0, ns, k):
            return pltpu.make_async_copy(obuf.at[pl.ds(s0, ns)], o_hbm.at[pl.ds(s0, ns)], osem.at[k])
        def wrh(q, h):
            sl = (pl.ds(4*q, 4), slice(None), pl.ds(512*h, 512))
            return pltpu.make_async_copy(obuf.at[sl], o_hbm.at[sl], osem.at[1 + 2*q + h])
        def wrblk(sl, k):
            return pltpu.make_async_copy(obuf.at[sl], o_hbm.at[sl], tsem.at[k])
        wcps = [pltpu.make_async_copy(w_hbm, wbuf, isem.at[NC + NQD]), pltpu.make_async_copy(g_hbm, g_ref, isem.at[NC + NQD + 1]),
                pltpu.make_async_copy(b_hbm, b_ref, isem.at[NC + NQD + 2])]
        for c in wcps: c.start()
        for i in range(2 if nord else NC): rdp(i).start()
        if not nord:
            for q in range(2, NQD): rdq(q).start()
        flag[0] = 1
        rid = lax.broadcasted_iota(jnp.int32,(KR - 64, 256),0)
        ones = pk((rid<2).astype(f32).astype(bf16))
        for t in range(4):
            for j in range(4): br[t, j, 32:KR//2, :] = ones
        for c in wcps: c.wait()
        prep_body(wbuf, g_ref, b_ref, af_ref, as_ref, ar_ref)

        cfg = dict(nacc=pnacc)
        def stats_item(sl, c0, slot, l0, width, j):
            s = sl[j]
            cols = slice(c0, c0 + width); lanes = slice(l0, l0 + width)
            k = width // 128
            ld = lambda r0: xbuf[s, r0:r0+8, cols].astype(f32)
            na = cfg['nacc'] * 2 // k
            def fold(accs, q, v): accs[q % na] = v if accs[q % na] is None else accs[q % na] + v
            tot = lambda accs: functools.reduce(lambda a, b: a + b, accs)
            if onepass and (width == 128 or mainop):
                na = max(na // 2, 1)
                NB = D // 8
                c = ld(0)
                s1 = [None] * na; s2 = [None] * na
                for q in range(1, NB):
                    d = ld(8*q) - c
                    fold(s1, q, d); fold(s2, q, d * d)
                    yield 5*k
                s1 = tot(s1); s2 = tot(s2)
                dm = s1 * (1.0 / NB)
                mj = c + dm
                m = jnp.broadcast_to(jnp.sum(mj, axis=0, keepdims=True) * 0.125, (8, width))
                e = mj - m
                m2 = (s2 - s1 * dm) + (e * e) * float(NB)
                var = jnp.maximum(jnp.sum(m2, axis=0, keepdims=True) * (1.0 / D), 0.0)
                sb[slot, j, 0, :, lanes] = m
            else:
                accs = [None] * na
                for q in range(D // 8):
                    fold(accs, q, ld(8*q))
                    yield 2*k
                m = jnp.broadcast_to(jnp.sum(tot(accs), axis=0, keepdims=True) * (1.0 / D), (8, width))
                sb[slot, j, 0, :, lanes] = m
                accs = [None] * na
                for q in range(D // 8):
                    v = ld(8*q) - m
                    fold(accs, q, v * v)
                    yield 4*k
                var = jnp.sum(tot(accs), axis=0, keepdims=True) * (1.0 / D)
            sb[slot, j, 1, :, lanes] = jnp.broadcast_to(lax.rsqrt(var + 1e-5), (8, width))

        def norm_item(sl, c0, slot, l0, q):
            cols = slice(c0, c0 + 128); lanes = slice(l0, l0 + 128)
            def nrm(j, r0):
                return (xbuf[sl[j], r0:r0+8, cols].astype(f32) - sb[slot, j, 0, :, lanes]) * sb[slot, j, 1, :, lanes]
            if q < KH // 16:
                gens = []
                for h in range(2):
                    r0 = 16*q + 8*h
                    gens.append(b_operands([nrm(j, r0) for j in range(4)], [nrm(j, KH + r0) for j in range(4)]))
                cuts = {1: [], 2: [(13, 90)], 3: [(7, 72), (16, 33)]}[nsub]
                done = 0
                for (k, v0), (_, v1) in zip(*gens):
                    bs[slot, k, 8*q:8*q+8, lanes] = pk2(v0, v1)
                    for kc, n in cuts:
                        if k == kc:
                            done += n; yield n
                yield N_OPS - done
            else:
                for j in range(4):
                    for qq in range(4):
                        r0 = 2*KH + 16*qq
                        br[slot, j, 8*qq:8*qq+8, lanes] = pk2(nrm(j, r0), nrm(j, r0 + 8))
                    yield 28

        class LN:
            def __init__(self, units):
                self.S = []; self.N = []
                for ui, (sl, c0, slot, l0, width) in enumerate(units):
                    for j in range(4): self.S.append((ui, (sl, c0, slot, l0, width, j), SOPS * width // 128))
                    for t in range(width // 128):
                        for q in range(KH // 16 + 1):
                            self.N.append((ui, (sl, c0 + 128*t, slot, l0 + 128*t, q), N_OPS if q < KH // 16 else 112))
                self.st = {u: sum(it[2] for it in self.S if it[0] == u) for u in range(len(units))}
                self.nt = {u: sum(it[2] for it in self.N if it[0] == u) for u in range(len(units))}
            def total(self): return sum(it[2] for it in self.S) + sum(it[2] for it in self.N)
            def take(self, budget, max_unit, need):
                seq = []; ops = 0
                slack = budget - sum(it[2] for it in self.S + self.N if it[0] <= need)
                tot = lambda L, u: sum(it[2] for it in L if it[0] == u)
                while True:
                    ok = lambda it: it[0] <= need or (it[0] <= max_unit and slack >= it[2])
                    s_ok = bool(self.S) and ok(self.S[0])
                    n_ok = bool(self.N) and ok(self.N[0]) and not (self.S and self.S[0][0] <= self.N[0][0])
                    if s_ok and self.N and self.S[0][0] > self.N[0][0] + 1: s_ok = False
                    if not (s_ok or n_ok): break
                    if s_ok and n_ok:
                        u = self.N[0][0]
                        pick_s = tot(self.S, u + 1) / self.st[u + 1] >= tot(self.N, u) / self.nt[u]
                    else: pick_s = s_ok
                    it = (self.S if pick_s else self.N).pop(0)
                    if it[0] > need: slack -= it[2]
                    seq.append((pick_s, it)); ops += it[2]
                def gen():
                    i = 0
                    while i < len(seq):
                        is_s, it = seq[i]
                        if not is_s:
                            yield from norm_item(*it[1]); i += 1; continue
                        g = stats_item(*it[1])
                        k = i + 1; follow = []
                        while k < len(seq) and not seq[k][0] and seq[k][1][0] < it[0]:
                            follow.append(seq[k][1]); k += 1
                        per = it[2] / (len(follow) + 1)
                        done = 0; fi = 0
                        for n in g:
                            done += n; yield n
                            if fi < len(follow) and done >= per * (fi + 1):
                                yield from norm_item(*follow[fi][1]); fi += 1
                        for f_ in follow[fi:]: yield from norm_item(*f_[1])
                        i = k
                return gen(), ops

        def mm_unit(unit, tp, tick, done, rows):
            sl, c0, slot, l0, width = unit
            cols = slice(c0, c0 + width); lanes = slice(l0, l0 + width); tl = slice(0, width)
            offs = np.cumsum((0,) + tuple(rows))
            def P(k):
                return lambda r: dot(up(as_ref[k, r.start//2:r.stop//2, :]), up(bs[slot, k, :, lanes]))
            def REM(i, j):
                return lambda r: dot(up(ar_ref[(NQ*i + r.start)//2:(NQ*i + r.stop)//2, :KR]), up(br[slot, j, :, lanes]))
            def rnd(post, fins=()):
                for c in range(len(rows)):
                    r = slice(int(offs[c]), int(offs[c+1]))
                    def st(k, v): tb[tp, k, r, tl] = v
                    def ld(k): return tb[tp, k, r, tl]
                    def fin(i, j, v): obuf[sl[j], NQ*i + r.start:NQ*i + r.stop, cols] = v.astype(bf16)
                    post(r, st, ld, fin)
                    tick(rows[c] / NQ * width / 256)
                for ij in fins: done(*ij)
            def raw(k, p): rnd(lambda r, st, ld, fin: st(k, p(r)))
            def diag(i): raw(i, P(i)); raw(4 + i, P(4 + i))
            def dfin(i, j):
                a = REM(i, i); b = REM(j, j)
                def post(r, st, ld, fin):
                    fin(i, i, a(r) + (ld(i) + ld(4 + i))); fin(j, j, b(r) + (ld(j) + ld(4 + j)))
                rnd(post, [(i, i), (j, j)])
            def pair(p):
                i, j = PAIRS[p]
                R, U1, U2 = 8 + 3*(p % 2), 9 + 3*(p % 2), 10 + 3*(p % 2)
                raw(R, P(8 + 3*p))
                a = REM(i, j); b = REM(j, i)
                def post(r, st, ld, fin):
                    st(U1, a(r) - (ld(i) + ld(4 + j))); st(U2, b(r) - (ld(j) + ld(4 + i)))
                rnd(post)
                q1 = P(9 + 3*p); rnd(lambda r, st, ld, fin: fin(i, j, q1(r) + (ld(U1) - ld(R))), [(i, j)])
                q2 = P(10 + 3*p); rnd(lambda r, st, ld, fin: fin(j, i, q2(r) + (ld(U2) + ld(R))), [(j, i)])
            diag(0); diag(1); dfin(0, 1); pair(0)
            diag(2); pair(1); pair(2)
            diag(3); dfin(2, 3); pair(3); pair(4); pair(5)

        def phase(mm_units, gen, total, rows, after_unit=lambda i: None, done=lambda u, i, j: None):
            wtot = sum(34 * u[4] / 256 for u in mm_units)
            quota = max(total - lead - trail, 0) / wtot
            state = dict(debt=0)
            def tick(w=None, n=None):
                state['debt'] += quota * w if n is None else n
                while state['debt'] > 0:
                    try: state['debt'] -= next(gen)
                    except StopIteration: return
            if lead: tick(n=lead)
            for i, u in enumerate(mm_units):
                mm_unit(u, i % 2, tick, functools.partial(done, i), rows)
                after_unit(i)
            for _ in gen: pass

        q0 = [0, 1, 2, 3]; q1 = [4, 5, 6, 7]
        hu = [(q0, 128*t, t // 2, 128*(t % 2), 128) for t in range(4)]
        g2, g3 = (q0, 512, 2, 0, 256), (q0, 768, 3, 0, 256)
        n0, n1 = (q1, 0, 0, 0, 256), (q1, 256, 1, 0, 256)
        ln = LN(hu + [g2, g3, n0, n1])
        HU = 4*SOPS + 16*N_OPS + 112
        rdp(0).wait()
        @pl.when(flag[0] == 1)
        def _():
            gens = [stats_item(*ln.S.pop(0)[1]) for _ in range(4)]
            for _ in itertools.zip_longest(*gens): pass
        for part in range(psplit):
            @pl.when(flag[0] == 1)
            def _():
                n = [it for it in ln.N if it[0] == 0]
                for it in n[:(len(n) + psplit - part - 1) // (psplit - part)]:
                    ln.N.remove(it)
                    for _ in norm_item(*it[1]): pass
        cfg['nacc'] = hnacc
        head = [([hu[0]], [1], 1), ([hu[1]], [2], 3), ([hu[2]], [3], 4), ([hu[3]], [4], 5), ([g2], [5], 6), ([g3], [6], 7)]
        need_done = [1, 2, 3, 4, 5, 7]
        for k, (mmu, waits, maxu) in enumerate(head):
            for wi in waits:
                if not (nord and wi >= 2): rdp(wi).wait()
            g_, ops = ln.take(plan[k] * HU, maxu, need_done[k])
            if verbose: print('head phase', k, ops / HU)
            assert not any(it[0] <= need_done[k] for it in ln.S + ln.N), k
            pl.when(flag[0] == 1)(functools.partial(phase, mmu, g_, ops, hrows))
        cfg['nacc'] = nacc
        cl = lambda s: jnp.minimum(s, S - 1)
        tails = []
        def body(q, carry):
            s0 = 4*q
            cur = [s0 + j for j in range(4)]
            sc = [cl(s0 + j) for j in range(4)]
            sn = [cl(s0 + 4 + j) for j in range(4)]
            if not nord:
                @pl.when(q == 1)
                def _(): rdp(NC - 1).wait()
            if not nowr and not JB:
                @pl.when(q == J0)
                def _(): wrs(0, 4*J0, 0).start()
            @pl.when(flag[0] == 1)
            def _():
                l = LN([(sc, 512, 2, 0, 256), (sc, 768, 3, 0, 256)])
                g_, ops = l.take(0, 9, 9)
                phase([(cur, 0, 0, 0, 256), (cur, 256, 1, 0, 256)], g_, ops, rows)
            if not nowr:
                if JB:
                    @pl.when(q == J0)
                    def _(): wrs(0, 4*J0, 0).start()
                @pl.when(q >= J0)
                def _(): wrh(q, 0).start()
            if not nord:
                @pl.when(q < NQD - 1)
                def _(): rdq(q + 1).wait()
            @pl.when(q < (NQD - 1) * flag[0])
            def _():
                l = LN([(sn, 0, 0, 0, 256), (sn, 256, 1, 0, 256)])
                g_, ops = l.take(0, 9, 9)
                phase([(cur, 512, 2, 0, 256), (cur, 768, 3, 0, 256)], g_, ops, rows)
            if not nowr:
                @pl.when(jnp.logical_and(q >= J0, q < NQD - 1))
                def _(): wrh(q, 1).start()
            return carry
        lax.fori_loop(1, NQD, body, 0)
        def go(sl):
            c = wrblk(sl, 1 + len(tails)); c.start(); tails.append(c)
        def au_last(i):
            if nowr or notail or i == 1 or tailmode == 3: return
            go((pl.ds(S - 4, 4), slice(None), pl.ds(512, 256)))
        def done_last(u, i, j):
            if nowr or notail: return
            cols = pl.ds(512 + 256*u, 256)
            if tailmode == 0:
                if u == 1: go((S - 4 + j, pl.ds(NQ*i, NQ), cols))
                return
            if u == 0 and tailmode in (1, 2): return
            if (i, j) == (1, 0) and tailmode >= 2: go((pl.ds(S - 4, 2), pl.ds(0, 2*NQ), cols))
            if (i, j) == (3, 3):
                if tailmode >= 2:
                    go((S - 2, pl.ds(0, 3*NQ), cols)); go((pl.ds(S - 4, 2), pl.ds(2*NQ, NQ), cols))
                else:
                    go((pl.ds(S - 4, 3), pl.ds(0, 3*NQ), cols))
                go((S - 1, pl.ds(3*NQ, NQ), cols))
            if (i, j) == (3, 1):
                go((S - 1, pl.ds(0, 2*NQ), cols)); go((pl.ds(S - 4, 2), pl.ds(3*NQ, NQ), cols))
            if (i, j) == (2, 3): go((S - 1, pl.ds(2*NQ, NQ), cols))
            if (i, j) == (3, 2): go((S - 2, pl.ds(3*NQ, NQ), cols))
        ql = [S - 4 + j for j in range(4)]
        phase([(ql, 512, 2, 0, 256), (ql, 768, 3, 0, 256)], iter(()), 0, (NQ,), au_last, done_last)
        if not nowr:
            wrs(0, 4*J0, 0).wait()
            for q in range(J0, NQD):
                wrh(q, 0).wait()
                if q < NQD - 1: wrh(q, 1).wait()
            for c in tails: c.wait()

    def f(x, g, b, w):
        xt = jnp.transpose(x, (1, 2, 0))
        out = pl.pallas_call(
            kern,
            in_specs=[pl.BlockSpec(memory_space=pl.ANY)] * 4,
            out_specs=pl.BlockSpec(memory_space=pl.ANY),
            out_shape=jax.ShapeDtypeStruct((S, D, B), x.dtype),
            scratch_shapes=[pltpu.VMEM((S, D, B), bf16), pltpu.VMEM((S, D, B), bf16), pltpu.VMEM((D, D), bf16),
                            pltpu.VMEM((D,), bf16), pltpu.VMEM((D,), bf16), pltpu.VMEM((5, D, 128), f32),
                            pltpu.VMEM((26, NQ//2, KH), u32), pltpu.VMEM((D//2, 128), u32),
                            pltpu.VMEM((4, 26, KH//2, 256), u32), pltpu.VMEM((4, 4, KR//2, 256), u32),
                            pltpu.VMEM((2, 14, NQ, 256), f32), pltpu.VMEM((4, 4, 2, 8, 256), f32), pltpu.SMEM((1,), jnp.int32),
                            pltpu.SemaphoreType.DMA((8 + NQD + 3,)), pltpu.SemaphoreType.DMA((2*NQD + 1,)),
                            pltpu.SemaphoreType.DMA((20,))],
            compiler_params=pltpu.CompilerParams(vmem_limit_bytes=120*1024*1024,
                disable_bounds_checks=not checks, disable_semaphore_checks=not checks),
        )(xt, w, g, b)
        return jnp.transpose(out, (2, 0, 1))
    return f

_impl = make()

@jax.jit
def pallas_standalone__layernorm_linear__sampling_kernel(x, g, b, w):
    return _impl(x, g, b, w)
```

```python
import functools
import itertools

import jax
import jax.numpy as jnp
from jax import lax
import jax.experimental.pallas as pl
import jax.experimental.pallas.tpu as pltpu

f32 = jnp.float32
bf16 = jnp.bfloat16
u32 = jnp.uint32

S, D, B = 32, 576, 1024
KH = 256
NH, NQ = 288, 144
KR = 80
NP = S // 2
EPS = 1e-5

SWAP = (False, True, False, False, True, True, True)

STATS_OPS, NORM_OPS, REM_OPS = 710, 255, 112
UNIT_OPS = 2 * STATS_OPS + 8 * NORM_OPS + REM_OPS


def _as_bf16(v):
    return pltpu.bitcast(v, bf16)


def _dot(a, b):
    return jnp.dot(a, b, preferred_element_type=f32)


def _add(x, y):
    return x + y


def _sub(x, y):
    return x - y


def _add2(a, b):
    return [[a[i][j] + b[i][j] for j in range(2)] for i in range(2)]


def _sub2(a, b):
    return [[a[i][j] - b[i][j] for j in range(2)] for i in range(2)]


def _strassen_lhs(a, add, sub):
    (a11, a12), (a21, a22) = a
    return [add(a11, a22), add(a21, a22), a11, a22, add(a11, a12), sub(a21, a11), sub(a12, a22)]


def _strassen_rhs(b):
    (b11, b12), (b21, b22) = b
    return [b11 + b22, b11, b12 - b22, b21 - b11, b22, b11 + b12, b21 + b22]


def _prepare_weights(w_ref, g_ref, b_ref, af_ref, as_ref, ar_ref):
    g_row = g_ref[...].astype(f32).reshape(1, D)
    b_row = b_ref[...].astype(f32).reshape(1, D)
    w = w_ref[...]
    rid = lax.broadcasted_iota(jnp.int32, (16, D), 0)
    bmat = jnp.where(rid < 2, jnp.broadcast_to(b_row, (16, D)), 0.0).astype(bf16)
    bias = _dot(bmat, w)
    hi = bias.astype(bf16).astype(f32)
    extra = jnp.where(rid == 0, hi, bias - hi)
    waug = jnp.concatenate([w.astype(f32), extra, jnp.zeros((48, D), f32)], axis=0)
    waug = jnp.concatenate([waug, jnp.zeros((640, 64), f32)], axis=1)
    gaug = jnp.concatenate([g_row, jnp.ones((1, 64), f32)], axis=1)
    a = waug.T[:D] * gaug
    for kt in range(4):
        af_ref[kt] = a[:, 128 * kt:128 * (kt + 1)]
    ar_ref[...] = a[:, 2 * KH:].astype(bf16)
    for q in range(NQ // 16):
        def blk(i2, k2):
            return [[af_ref[2 * k2 + k, pl.ds(NQ * (2 * i2 + i) + 16 * q, 16), :] for k in range(2)]
                    for i in range(2)]
        outer = _strassen_lhs([[blk(0, 0), blk(0, 1)], [blk(1, 0), blk(1, 1)]], _add2, _sub2)
        for o in range(7):
            for n, v in enumerate(_strassen_lhs(outer[o], _add, _sub)):
                as_ref[7 * o + n, 16 * q:16 * q + 16, :] = v.astype(bf16)


MAIN_KNOBS = dict(lead=100, trail=-250, wrem=1.5, wfin=1.0, tk=1)
HEAD_KNOBS = (
    dict(lead=300, trail=0, wrem=1.5, wfin=0.7, tk=2),
    dict(lead=130, trail=-350, wrem=1.22, wfin=1.01, tk=1),
    dict(lead=0, trail=-100, wrem=1.0, wfin=0.6, tk=2),
    dict(lead=200, trail=-50, wrem=0.94, wfin=0.63, tk=1),
    dict(lead=50, trail=-200, wrem=1.35, wfin=0.8, tk=2),
    dict(lead=60, trail=-100, wrem=1.18, wfin=0.68, tk=2),
)
HEAD_PLAN = (1.0, 1.33, 1.33, 1.33, 3.0, 3.0)
RC = 48
WRITE_FROM = 7
WCOLS = 128


def _kernel(x_hbm, w_hbm, g_hbm, b_hbm, o_hbm,
            xbuf, obuf, wbuf, g_ref, b_ref, af_ref, as_ref, ar_ref, bs, br, tb, sb, flag,
            isem, osem, tsem):
    as_u, ar_u, bs_u, br_u = (r.bitcast(u32) for r in (as_ref, ar_ref, bs, br))

    chunks = [(0, 0, 256), (0, 256, 256), (0, 512, 512), (2, 0, 512), (2, 512, 512),
              (4, 0, 512), (4, 512, 512)]
    nch = len(chunks)

    def read_chunk(i):
        s0, c0, nc = chunks[i]
        sl = (pl.ds(s0, 2), slice(None), pl.ds(c0, nc))
        return pltpu.make_async_copy(x_hbm.at[sl], xbuf.at[sl], isem.at[i])

    def read_pair(p):
        return pltpu.make_async_copy(x_hbm.at[pl.ds(2 * p, 2)], xbuf.at[pl.ds(2 * p, 2)], isem.at[nch + p])

    def write_slices(s0, ns, k):
        sls = [(pl.ds(s0, ns), slice(None), pl.ds(c, WCOLS)) for c in range(0, B, WCOLS)]
        return [pltpu.make_async_copy(obuf.at[sl], o_hbm.at[sl], osem.at[k]) for sl in sls]

    param_copies = [pltpu.make_async_copy(src, dst, isem.at[nch + NP + i])
                    for i, (src, dst) in enumerate(((w_hbm, wbuf), (g_hbm, g_ref), (b_hbm, b_ref)))]
    for c in param_copies:
        c.start()
    for i in range(nch):
        read_chunk(i).start()
    for p in range(3, NP):
        read_pair(p).start()

    flag[0] = 1
    rid = lax.broadcasted_iota(jnp.int32, (KR - 64, 128), 0)
    ones = (rid < 2).astype(f32).astype(bf16)
    for t in range(8):
        for j in range(2):
            for h in range(2):
                br[t, j, h, 64:KR, :] = ones
    for c in param_copies:
        c.wait()
    _prepare_weights(wbuf, g_ref, b_ref, af_ref, as_ref, ar_ref)

    def stats_item(sl, g, slot, j):
        cols = slice(256 * g, 256 * g + 256)
        ld = lambda q: xbuf[sl[j], 8 * q:8 * q + 8, cols].astype(f32)
        nb = D // 8
        c = ld(0)
        s1 = s2 = None
        for q in range(1, nb):
            d = ld(q) - c
            s1 = d if s1 is None else s1 + d
            s2 = d * d if s2 is None else s2 + d * d
            yield 10
        dm = s1 * (1.0 / nb)
        mj = c + dm
        m = jnp.sum(mj, axis=0, keepdims=True) * 0.125
        e = mj - m
        m2 = (s2 - s1 * dm) + (e * e) * float(nb)
        var = jnp.maximum(jnp.sum(m2, axis=0, keepdims=True) * (1.0 / D), 0.0)
        sb[slot, j, 0:1, :] = m
        sb[slot, j, 1:2, :] = lax.rsqrt(var + EPS)

    def norm_item(sl, g, slot, q):
        cols = slice(256 * g, 256 * g + 256)

        def nrm(j, r0, n=16):
            return (xbuf[sl[j], r0:r0 + n, cols].astype(f32) - sb[slot, j, 0:1, :]) * sb[slot, j, 1:2, :]

        if q == 8:
            for j in range(2):
                v = nrm(j, 2 * KH, 64)
                br[slot, j, 0, 0:64, :] = v[:, :128].astype(bf16)
                br[slot, j, 1, 0:64, :] = v[:, 128:].astype(bf16)
                yield 56
            return

        def blk(k2, j):
            return [[v[:, :128], v[:, 128:]] for v in (nrm(j, KH * k2 + 128 * k + 16 * q) for k in range(2))]

        def emit(o, b):
            if SWAP[o]:
                b = [[b[0][1], b[0][0]], [b[1][1], b[1][0]]]
            for n, v in enumerate(_strassen_rhs(b)):
                bs[slot, 7 * o + n, 16 * q:16 * q + 16, :] = v.astype(bf16)

        b11 = blk(0, 0)
        emit(1, b11)
        yield 41
        b12 = blk(0, 1)
        emit(5, _add2(b11, b12))
        yield 49
        b22 = blk(1, 1)
        emit(2, _sub2(b12, b22))
        yield 49
        emit(0, _add2(b11, b22))
        yield 25
        emit(4, b22)
        yield 17
        b21 = blk(1, 0)
        emit(3, _sub2(b21, b11))
        yield 49
        emit(6, _add2(b21, b22))
        yield 25

    class LnQueue:
        def __init__(self, units):
            self.stats = [(u, (sl, g, slot, j), STATS_OPS)
                          for u, (sl, g, slot) in enumerate(units) for j in range(2)]
            self.norm = [(u, (sl, g, slot, q), NORM_OPS if q < 8 else REM_OPS)
                         for u, (sl, g, slot) in enumerate(units) for q in range(9)]

        def take(self, budget, max_unit, need):
            st, nm = self.stats, self.norm
            slack = budget - sum(it[2] for it in st + nm if it[0] <= need)
            left = lambda items, u: sum(it[2] for it in items if it[0] == u)
            seq = []
            while True:
                ok = lambda it: it[0] <= need or (it[0] <= max_unit and slack >= it[2])
                s_ok = bool(st) and ok(st[0]) and not (nm and st[0][0] > nm[0][0] + 1)
                n_ok = bool(nm) and ok(nm[0]) and not (st and st[0][0] <= nm[0][0])
                if not (s_ok or n_ok):
                    break
                if s_ok and n_ok:
                    u = nm[0][0]
                    s_ok = left(st, u + 1) / (2 * STATS_OPS) >= left(nm, u) / (8 * NORM_OPS + REM_OPS)
                it = (st if s_ok else nm).pop(0)
                if it[0] > need:
                    slack -= it[2]
                seq.append((s_ok, it))
            assert not any(it[0] <= need for it in st + nm)

            def gen():
                i = 0
                while i < len(seq):
                    is_stats, it = seq[i]
                    i += 1
                    if not is_stats:
                        yield from norm_item(*it[1])
                        continue
                    follow = []
                    while i < len(seq) and not seq[i][0] and seq[i][1][0] < it[0]:
                        follow.append(seq[i][1])
                        i += 1
                    ng = itertools.chain.from_iterable(norm_item(*f[1]) for f in follow)
                    ntot = sum(f[2] for f in follow)
                    ds = dn = 0
                    for n in stats_item(*it[1]):
                        ds += n
                        yield n
                        while dn * it[2] < ds * ntot:
                            m = next(ng, None)
                            if m is None:
                                break
                            dn += m
                            yield m
                    yield from ng

            return gen(), sum(it[2] for _, it in seq)

    def mm_unit(unit, tp, tick, done, kn):
        sl, g, slot = unit
        cols = slice(256 * g, 256 * g + 256)
        wtot = 35 + 14 * kn['wfin'] + 16 * kn['wrem']

        def prod(o, post):
            w = RC / NQ / wtot * (kn['wfin'] if o >= 5 else 1.0)
            for r0 in range(0, NQ, RC):
                p = lambda n: _dot(_as_bf16(as_u[7 * o + n - 1, r0 // 2:(r0 + RC) // 2, :]),
                                   _as_bf16(bs_u[slot, 7 * o + n - 1]))
                p5, p3 = p(5), p(3)
                if kn['tk'] == 2:
                    tick(2 * w)
                p1, p7 = p(1), p(7)
                t12, t11, t22 = p5 + p3, (p1 + p7) - p5, p1 + p3
                tick(2 * w if kn['tk'] == 2 else 4 * w)
                p4, p2, p6 = p(4), p(2), p(6)
                t11, t21, t22 = t11 + p4, p2 + p4, t22 + (p6 - p2)
                if SWAP[o]:
                    t11, t12, t21, t22 = t12, t11, t22, t21
                top, bot = jnp.concatenate([t11, t12], axis=1), jnp.concatenate([t21, t22], axis=1)
                post(slice(r0, r0 + RC), top)
                post(slice(NQ + r0, NQ + r0 + RC), bot)
                tick(3 * w)

        def rem(i2, j, post):
            for r0 in range(0, NH, RC):
                v = _dot(_as_bf16(ar_u[(NH * i2 + r0) // 2:(NH * i2 + r0 + RC) // 2, :])[:, :KR],
                         jnp.concatenate([_as_bf16(br_u[slot, j, 0]), _as_bf16(br_u[slot, j, 1])], axis=1))
                post(slice(r0, r0 + RC), v)
                tick(kn['wrem'] * 2 * RC / NQ / wtot)

        def ld(k, r):
            return tb[tp, k, r, :]

        def keep(k):
            def post(r, v):
                tb[tp, k, r, :] = v
            return post

        def out(i2, j, r, v):
            obuf[sl[j], NH * i2 + r.start:NH * i2 + r.stop, cols] = v.astype(bf16)

        prod(1, keep(1))
        prod(3, keep(3))
        rem(1, 0, lambda r, v: out(1, 0, r, v + (ld(1, r) + ld(3, r))))
        done(1, 0)
        prod(2, keep(2))
        prod(4, keep(4))
        rem(0, 1, lambda r, v: out(0, 1, r, v + (ld(2, r) + ld(4, r))))
        done(0, 1)
        prod(0, keep(0))
        rem(0, 0, lambda r, v: keep(5)(r, (v + ld(0, r)) + (ld(3, r) - ld(4, r))))
        prod(6, lambda r, v: out(0, 0, r, v + ld(5, r)))
        done(0, 0)
        rem(1, 1, lambda r, v: keep(6)(r, (v + ld(0, r)) + (ld(2, r) - ld(1, r))))
        prod(5, lambda r, v: out(1, 1, r, v + ld(6, r)))
        done(1, 1)

    def phase(units, ln_gen, ln_ops, kn, done=lambda u, i2, j: None):
        quota = max(ln_ops - kn['lead'] - kn['trail'], 0) / len(units)
        debt = [0.0]

        def pay(n):
            debt[0] += n
            while debt[0] > 0:
                step = next(ln_gen, None)
                if step is None:
                    return
                debt[0] -= step

        pay(kn['lead'])
        for i, u in enumerate(units):
            mm_unit(u, i % 2, lambda w: pay(quota * w), functools.partial(done, i), kn)
        for _ in ln_gen:
            pass

    hu = [([2 * (u // 4), 2 * (u // 4) + 1], u % 4, u % 8) for u in range(12)]
    ln = LnQueue(hu)
    read_chunk(0).wait()

    @pl.when(flag[0] == 1)
    def _():
        for _ in itertools.zip_longest(*[stats_item(*ln.stats.pop(0)[1]) for _ in range(2)]):
            pass

    @pl.when(flag[0] == 1)
    def _():
        while ln.norm[0][0] == 0:
            for _ in norm_item(*ln.norm.pop(0)[1]):
                pass

    head = [(hu[0:1], 1, 1), (hu[1:2], 3, 2), (hu[2:3], 5, 3), (hu[3:4], 7, 5), (hu[4:6], 9, 7), (hu[6:8], 11, 11)]
    for k, (units, max_unit, need) in enumerate(head):
        read_chunk(k + 1).wait()
        gen, ops = ln.take(HEAD_PLAN[k] * UNIT_OPS, max_unit, need)
        pl.when(flag[0] == 1)(functools.partial(phase, units, gen, ops, HEAD_KNOBS[k]))

    def body(p, carry):
        cur = [2 * p, 2 * p + 1]
        nxt = [jnp.minimum(2 * p + 2, S - 1), jnp.minimum(2 * p + 3, S - 1)]
        read_pair(p + 1).wait()

        @pl.when(p == WRITE_FROM)
        def _():
            for c in write_slices(0, 2 * WRITE_FROM, 0):
                c.start()

        for par in range(2):
            @pl.when(p % 2 == par)
            def _():
                gen, ops = LnQueue([(nxt, g, 4 * (1 - par) + g) for g in range(4)]).take(0, 3, 3)
                phase([(cur, g, 4 * par + g) for g in range(4)], gen, ops, MAIN_KNOBS)

        @pl.when(p >= WRITE_FROM)
        def _():
            for c in write_slices(2 * p, 2, p):
                c.start()
        return carry

    lax.fori_loop(2, NP - 1, body, 0)

    tail = []

    def send(sl):
        c = pltpu.make_async_copy(obuf.at[sl], o_hbm.at[sl], tsem.at[len(tail)])
        c.start()
        tail.append(c)

    def done_last(u, i2, j):
        cols = pl.ds(256 * u, 256)
        if u == 3:
            send((S - 2 + j, pl.ds(NH * i2, NH), cols))
        elif (i2, j) == (1, 1):
            send((pl.ds(S - 2, 2), slice(None), cols))

    phase([([S - 2, S - 1], g, 4 + g) for g in range(4)], iter(()), 0, MAIN_KNOBS, done_last)

    for c in write_slices(0, 2 * WRITE_FROM, 0):
        c.wait()
    for p in range(WRITE_FROM, NP - 1):
        for c in write_slices(2 * p, 2, p):
            c.wait()
    for c in tail:
        c.wait()


@jax.jit
def pallas_standalone__layernorm_linear__sampling_kernel(
    x: jax.Array,
    g: jax.Array,
    b: jax.Array,
    w: jax.Array,
):
    assert x.shape == (B, S, D) and w.shape == (D, D)
    out = pl.pallas_call(
        _kernel,
        in_specs=[pl.BlockSpec(memory_space=pl.ANY)] * 4,
        out_specs=pl.BlockSpec(memory_space=pl.ANY),
        out_shape=jax.ShapeDtypeStruct((S, D, B), x.dtype),
        scratch_shapes=[
            pltpu.VMEM((S, D, B), bf16),
            pltpu.VMEM((S, D, B), bf16),
            pltpu.VMEM((D, D), bf16),
            pltpu.VMEM((D,), bf16),
            pltpu.VMEM((D,), bf16),
            pltpu.VMEM((4, D, 128), f32),
            pltpu.VMEM((49, NQ, 128), bf16),
            pltpu.VMEM((D, 128), bf16),
            pltpu.VMEM((8, 49, 128, 128), bf16),
            pltpu.VMEM((8, 2, 2, KR, 128), bf16),
            pltpu.VMEM((2, 7, NH, 256), f32),
            pltpu.VMEM((8, 2, 8, 256), f32),
            pltpu.SMEM((1,), jnp.int32),
            pltpu.SemaphoreType.DMA((7 + NP + 3,)),
            pltpu.SemaphoreType.DMA((NP,)),
            pltpu.SemaphoreType.DMA((7,)),
        ],
        compiler_params=pltpu.CompilerParams(
            vmem_limit_bytes=120 * 1024 * 1024,
            disable_bounds_checks=True,
            disable_semaphore_checks=True),
    )(jnp.transpose(x, (1, 2, 0)), w, g, b)
    return jnp.transpose(out, (2, 0, 1))
```

```python
import functools
import itertools

import jax
import jax.numpy as jnp
from jax import lax
import jax.experimental.pallas as pl
import jax.experimental.pallas.tpu as pltpu

f32 = jnp.float32
bf16 = jnp.bfloat16
u32 = jnp.uint32

S, D, B = 32, 576, 1024
KH = 256
NH, NQ = 288, 144
KR = 80
NP = S // 2
EPS = 1e-5

SWAP = (False, True, False, False, True, True, True)

STATS_OPS, NORM_OPS, REM_OPS = 710, 255, 112
UNIT_OPS = 2 * STATS_OPS + 8 * NORM_OPS + REM_OPS


def _as_bf16(v):
    return pltpu.bitcast(v, bf16)


def _dot(a, b):
    return jnp.dot(a, b, preferred_element_type=f32)


def _add(x, y):
    return x + y


def _sub(x, y):
    return x - y


def _add2(a, b):
    return [[a[i][j] + b[i][j] for j in range(2)] for i in range(2)]


def _sub2(a, b):
    return [[a[i][j] - b[i][j] for j in range(2)] for i in range(2)]


def _strassen_lhs(a, add, sub):
    (a11, a12), (a21, a22) = a
    return [add(a11, a22), add(a21, a22), a11, a22, add(a11, a12), sub(a21, a11), sub(a12, a22)]


def _strassen_rhs(b):
    (b11, b12), (b21, b22) = b
    return [b11 + b22, b11, b12 - b22, b21 - b11, b22, b11 + b12, b21 + b22]


def _prepare_weights(w_ref, g_ref, b_ref, af_ref, as_ref, ar_ref):
    g_row = g_ref[...].astype(f32).reshape(1, D)
    b_row = b_ref[...].astype(f32).reshape(1, D)
    w = w_ref[...]
    rid = lax.broadcasted_iota(jnp.int32, (16, D), 0)
    bmat = jnp.where(rid < 2, jnp.broadcast_to(b_row, (16, D)), 0.0).astype(bf16)
    bias = _dot(bmat, w)
    hi = bias.astype(bf16).astype(f32)
    extra = jnp.where(rid == 0, hi, bias - hi)
    waug = jnp.concatenate([w.astype(f32), extra, jnp.zeros((48, D), f32)], axis=0)
    waug = jnp.concatenate([waug, jnp.zeros((640, 64), f32)], axis=1)
    gaug = jnp.concatenate([g_row, jnp.ones((1, 64), f32)], axis=1)
    a = waug.T[:D] * gaug
    for kt in range(4):
        af_ref[kt] = a[:, 128 * kt:128 * (kt + 1)]
    ar_ref[...] = a[:, 2 * KH:].astype(bf16)
    for q in range(NQ // 16):
        def blk(i2, k2):
            return [[af_ref[2 * k2 + k, pl.ds(NQ * (2 * i2 + i) + 16 * q, 16), :] for k in range(2)]
                    for i in range(2)]
        outer = _strassen_lhs([[blk(0, 0), blk(0, 1)], [blk(1, 0), blk(1, 1)]], _add2, _sub2)
        for o in range(7):
            for n, v in enumerate(_strassen_lhs(outer[o], _add, _sub)):
                as_ref[7 * o + n, 16 * q:16 * q + 16, :] = v.astype(bf16)


MAIN_KNOBS = dict(lead=100, trail=-250, wrem=1.5, wfin=1.0, tk=1)
HEAD_KNOBS = (
    dict(lead=300, trail=0, wrem=1.5, wfin=0.7, tk=2),
    dict(lead=130, trail=-350, wrem=1.22, wfin=1.01, tk=1),
    dict(lead=0, trail=-100, wrem=1.0, wfin=0.6, tk=2),
    dict(lead=200, trail=-50, wrem=0.94, wfin=0.63, tk=1),
    dict(lead=50, trail=-200, wrem=1.35, wfin=0.8, tk=2),
    dict(lead=60, trail=-100, wrem=1.18, wfin=0.68, tk=2),
)
HEAD_PLAN = (1.0, 1.33, 1.33, 1.33, 3.0, 3.0)
RC = 48
WRITE_FROM = 7
WCOLS = 128
BCOLS = 256


def _kernel(x_hbm, w_hbm, g_hbm, b_hbm, o_hbm,
            xbuf, obuf, wbuf, g_ref, b_ref, af_ref, as_ref, ar_ref, bs, br, tb, sb, flag,
            isem, osem, tsem):
    as_u, ar_u, bs_u, br_u = (r.bitcast(u32) for r in (as_ref, ar_ref, bs, br))

    chunks = [(0, 0, 256), (0, 256, 256), (0, 512, 512), (2, 0, 512), (2, 512, 512),
              (4, 0, 512), (4, 512, 512)]
    nch = len(chunks)

    def read_chunk(i):
        s0, c0, nc = chunks[i]
        sl = (pl.ds(s0, 2), slice(None), pl.ds(c0, nc))
        return pltpu.make_async_copy(x_hbm.at[sl], xbuf.at[sl], isem.at[i])

    def read_pair(p):
        return pltpu.make_async_copy(x_hbm.at[pl.ds(2 * p, 2)], xbuf.at[pl.ds(2 * p, 2)], isem.at[nch + p])

    def write_slices(s0, ns, k, wc=WCOLS):
        sls = [(pl.ds(s0, ns), slice(None), pl.ds(c, wc)) for c in range(0, B, wc)]
        return [pltpu.make_async_copy(obuf.at[sl], o_hbm.at[sl], osem.at[k]) for sl in sls]

    param_copies = [pltpu.make_async_copy(src, dst, isem.at[nch + NP + i])
                    for i, (src, dst) in enumerate(((w_hbm, wbuf), (g_hbm, g_ref), (b_hbm, b_ref)))]
    for c in param_copies:
        c.start()
    for i in range(nch):
        read_chunk(i).start()
    for p in range(3, NP):
        read_pair(p).start()

    flag[0] = 1
    rid = lax.broadcasted_iota(jnp.int32, (KR - 64, 128), 0)
    ones = (rid < 2).astype(f32).astype(bf16)
    for t in range(8):
        for j in range(2):
            for h in range(2):
                br[t, j, h, 64:KR, :] = ones
    for c in param_copies:
        c.wait()
    _prepare_weights(wbuf, g_ref, b_ref, af_ref, as_ref, ar_ref)

    def stats_item(sl, g, slot, j):
        cols = slice(256 * g, 256 * g + 256)
        ld = lambda q: xbuf[sl[j], 8 * q:8 * q + 8, cols].astype(f32)
        nb = D // 8
        c = ld(0)
        s1 = s2 = None
        for q in range(1, nb):
            d = ld(q) - c
            s1 = d if s1 is None else s1 + d
            s2 = d * d if s2 is None else s2 + d * d
            yield 10
        dm = s1 * (1.0 / nb)
        mj = c + dm
        m = jnp.sum(mj, axis=0, keepdims=True) * 0.125
        e = mj - m
        m2 = (s2 - s1 * dm) + (e * e) * float(nb)
        var = jnp.maximum(jnp.sum(m2, axis=0, keepdims=True) * (1.0 / D), 0.0)
        sb[slot, j, 0:1, :] = m
        sb[slot, j, 1:2, :] = lax.rsqrt(var + EPS)

    def norm_item(sl, g, slot, q):
        cols = slice(256 * g, 256 * g + 256)

        def nrm(j, r0, n=16):
            return (xbuf[sl[j], r0:r0 + n, cols].astype(f32) - sb[slot, j, 0:1, :]) * sb[slot, j, 1:2, :]

        if q == 8:
            for j in range(2):
                v = nrm(j, 2 * KH, 64)
                br[slot, j, 0, 0:64, :] = v[:, :128].astype(bf16)
                br[slot, j, 1, 0:64, :] = v[:, 128:].astype(bf16)
                yield 56
            return

        def blk(k2, j):
            return [[v[:, :128], v[:, 128:]] for v in (nrm(j, KH * k2 + 128 * k + 16 * q) for k in range(2))]

        def emit(o, b):
            if SWAP[o]:
                b = [[b[0][1], b[0][0]], [b[1][1], b[1][0]]]
            for n, v in enumerate(_strassen_rhs(b)):
                bs[slot, 7 * o + n, 16 * q:16 * q + 16, :] = v.astype(bf16)

        b11 = blk(0, 0)
        emit(1, b11)
        yield 41
        b12 = blk(0, 1)
        emit(5, _add2(b11, b12))
        yield 49
        b22 = blk(1, 1)
        emit(2, _sub2(b12, b22))
        yield 49
        emit(0, _add2(b11, b22))
        yield 25
        emit(4, b22)
        yield 17
        b21 = blk(1, 0)
        emit(3, _sub2(b21, b11))
        yield 49
        emit(6, _add2(b21, b22))
        yield 25

    class LnQueue:
        def __init__(self, units):
            self.stats = [(u, (sl, g, slot, j), STATS_OPS)
                          for u, (sl, g, slot) in enumerate(units) for j in range(2)]
            self.norm = [(u, (sl, g, slot, q), NORM_OPS if q < 8 else REM_OPS)
                         for u, (sl, g, slot) in enumerate(units) for q in range(9)]

        def take(self, budget, max_unit, need):
            st, nm = self.stats, self.norm
            slack = budget - sum(it[2] for it in st + nm if it[0] <= need)
            left = lambda items, u: sum(it[2] for it in items if it[0] == u)
            seq = []
            while True:
                ok = lambda it: it[0] <= need or (it[0] <= max_unit and slack >= it[2])
                s_ok = bool(st) and ok(st[0]) and not (nm and st[0][0] > nm[0][0] + 1)
                n_ok = bool(nm) and ok(nm[0]) and not (st and st[0][0] <= nm[0][0])
                if not (s_ok or n_ok):
                    break
                if s_ok and n_ok:
                    u = nm[0][0]
                    s_ok = left(st, u + 1) / (2 * STATS_OPS) >= left(nm, u) / (8 * NORM_OPS + REM_OPS)
                it = (st if s_ok else nm).pop(0)
                if it[0] > need:
                    slack -= it[2]
                seq.append((s_ok, it))
            assert not any(it[0] <= need for it in st + nm)

            def gen():
                i = 0
                while i < len(seq):
                    is_stats, it = seq[i]
                    i += 1
                    if not is_stats:
                        yield from norm_item(*it[1])
                        continue
                    follow = []
                    while i < len(seq) and not seq[i][0] and seq[i][1][0] < it[0]:
                        follow.append(seq[i][1])
                        i += 1
                    ng = itertools.chain.from_iterable(norm_item(*f[1]) for f in follow)
                    ntot = sum(f[2] for f in follow)
                    ds = dn = 0
                    for n in stats_item(*it[1]):
                        ds += n
                        yield n
                        while dn * it[2] < ds * ntot:
                            m = next(ng, None)
                            if m is None:
                                break
                            dn += m
                            yield m
                    yield from ng

            return gen, sum(it[2] for _, it in seq)

    def mm_unit(unit, tp, tick, done, kn):
        sl, g, slot = unit
        cols = slice(256 * g, 256 * g + 256)
        wtot = 35 + 14 * kn['wfin'] + 16 * kn['wrem']

        def prod(o, post):
            w = RC / NQ / wtot * (kn['wfin'] if o >= 5 else 1.0)
            for r0 in range(0, NQ, RC):
                p = lambda n: _dot(_as_bf16(as_u[7 * o + n - 1, r0 // 2:(r0 + RC) // 2, :]),
                                   _as_bf16(bs_u[slot, 7 * o + n - 1]))
                p5, p3 = p(5), p(3)
                if kn['tk'] == 2:
                    tick(2 * w)
                p1, p7 = p(1), p(7)
                t12, t11, t22 = p5 + p3, (p1 + p7) - p5, p1 + p3
                tick(2 * w if kn['tk'] == 2 else 4 * w)
                p4, p2, p6 = p(4), p(2), p(6)
                t11, t21, t22 = t11 + p4, p2 + p4, t22 + (p6 - p2)
                if SWAP[o]:
                    t11, t12, t21, t22 = t12, t11, t22, t21
                top, bot = jnp.concatenate([t11, t12], axis=1), jnp.concatenate([t21, t22], axis=1)
                post(slice(r0, r0 + RC), top)
                post(slice(NQ + r0, NQ + r0 + RC), bot)
                tick(3 * w)

        def rem(i2, j, post):
            for r0 in range(0, NH, RC):
                v = _dot(_as_bf16(ar_u[(NH * i2 + r0) // 2:(NH * i2 + r0 + RC) // 2, :])[:, :KR],
                         jnp.concatenate([_as_bf16(br_u[slot, j, 0]), _as_bf16(br_u[slot, j, 1])], axis=1))
                post(slice(r0, r0 + RC), v)
                tick(kn['wrem'] * 2 * RC / NQ / wtot)

        def ld(k, r):
            return tb[tp, k, r, :]

        def keep(k):
            def post(r, v):
                tb[tp, k, r, :] = v
            return post

        def out(i2, j, r, v):
            obuf[sl[j], NH * i2 + r.start:NH * i2 + r.stop, cols] = v.astype(bf16)

        prod(1, keep(1))
        prod(3, keep(3))
        rem(1, 0, lambda r, v: out(1, 0, r, v + (ld(1, r) + ld(3, r))))
        done(1, 0)
        prod(2, keep(2))
        prod(4, keep(4))
        rem(0, 1, lambda r, v: out(0, 1, r, v + (ld(2, r) + ld(4, r))))
        done(0, 1)
        prod(0, keep(0))
        rem(0, 0, lambda r, v: keep(5)(r, (v + ld(0, r)) + (ld(3, r) - ld(4, r))))
        prod(6, lambda r, v: out(0, 0, r, v + ld(5, r)))
        done(0, 0)
        rem(1, 1, lambda r, v: keep(6)(r, (v + ld(0, r)) + (ld(2, r) - ld(1, r))))
        prod(5, lambda r, v: out(1, 1, r, v + ld(6, r)))
        done(1, 1)

    def phase(units, make_ln_gen, ln_ops, kn, done=lambda u, i2, j: None):
        ln_gen = make_ln_gen()
        quota = max(ln_ops - kn['lead'] - kn['trail'], 0) / len(units)
        debt = [0.0]

        def pay(n):
            debt[0] += n
            while debt[0] > 0:
                step = next(ln_gen, None)
                if step is None:
                    return
                debt[0] -= step

        pay(kn['lead'])
        for i, u in enumerate(units):
            mm_unit(u, i % 2, lambda w: pay(quota * w), functools.partial(done, i), kn)
        for _ in ln_gen:
            pass

    hu = [([2 * (u // 4), 2 * (u // 4) + 1], u % 4, u % 8) for u in range(12)]
    ln = LnQueue(hu)
    read_chunk(0).wait()

    first_stats = [ln.stats.pop(0) for _ in range(2)]
    first_norm = [ln.norm.pop(0) for _ in range(9)]

    @pl.when(flag[0] == 1)
    def _():
        for _ in itertools.zip_longest(*[stats_item(*it[1]) for it in first_stats]):
            pass

    @pl.when(flag[0] == 1)
    def _():
        for it in first_norm:
            for _ in norm_item(*it[1]):
                pass

    head = [(hu[0:1], 1, 1), (hu[1:2], 3, 2), (hu[2:3], 5, 3), (hu[3:4], 7, 5), (hu[4:6], 9, 7), (hu[6:8], 11, 11)]
    for k, (units, max_unit, need) in enumerate(head):
        read_chunk(k + 1).wait()
        gen, ops = ln.take(HEAD_PLAN[k] * UNIT_OPS, max_unit, need)
        pl.when(flag[0] == 1)(functools.partial(phase, units, gen, ops, HEAD_KNOBS[k]))

    def body(p, carry):
        cur = [2 * p, 2 * p + 1]
        nxt = [jnp.minimum(2 * p + 2, S - 1), jnp.minimum(2 * p + 3, S - 1)]
        read_pair(p + 1).wait()

        for par in range(2):
            @pl.when((p & 1) == par)
            def _():
                gen, ops = LnQueue([(nxt, g, 4 * (1 - par) + g) for g in range(4)]).take(0, 3, 3)
                phase([(cur, g, 4 * par + g) for g in range(4)], gen, ops, MAIN_KNOBS)
                if par == (WRITE_FROM - 1) % 2:
                    @pl.when(p == WRITE_FROM - 1)
                    def _():
                        for c in write_slices(0, 2 * WRITE_FROM, 0, BCOLS):
                            c.start()

                @pl.when(p >= WRITE_FROM)
                def _():
                    for c in write_slices(2 * p, 2, p):
                        c.start()
        return carry

    lax.fori_loop(2, NP - 1, body, 0)

    tail = []

    def send(sl):
        c = pltpu.make_async_copy(obuf.at[sl], o_hbm.at[sl], tsem.at[len(tail)])
        c.start()
        tail.append(c)

    def done_last(u, i2, j):
        cols = pl.ds(256 * u, 256)
        if u == 3:
            send((S - 2 + j, pl.ds(NH * i2, NH), cols))
        elif (i2, j) == (1, 1):
            send((pl.ds(S - 2, 2), slice(None), cols))

    phase([([S - 2, S - 1], g, 4 + g) for g in range(4)], lambda: iter(()), 0, MAIN_KNOBS, done_last)

    for c in write_slices(0, 2 * WRITE_FROM, 0, BCOLS):
        c.wait()
    for p in range(WRITE_FROM, NP - 1):
        for c in write_slices(2 * p, 2, p):
            c.wait()
    for c in tail:
        c.wait()


@jax.jit
def pallas_standalone__layernorm_linear__sampling_kernel(
    x: jax.Array,
    g: jax.Array,
    b: jax.Array,
    w: jax.Array,
):
    assert x.shape == (B, S, D) and w.shape == (D, D)
    out = pl.pallas_call(
        _kernel,
        in_specs=[pl.BlockSpec(memory_space=pl.ANY)] * 4,
        out_specs=pl.BlockSpec(memory_space=pl.ANY),
        out_shape=jax.ShapeDtypeStruct((S, D, B), x.dtype),
        scratch_shapes=[
            pltpu.VMEM((S, D, B), bf16),
            pltpu.VMEM((S, D, B), bf16),
            pltpu.VMEM((D, D), bf16),
            pltpu.VMEM((D,), bf16),
            pltpu.VMEM((D,), bf16),
            pltpu.VMEM((4, D, 128), f32),
            pltpu.VMEM((49, NQ, 128), bf16),
            pltpu.VMEM((D, 128), bf16),
            pltpu.VMEM((8, 49, 128, 128), bf16),
            pltpu.VMEM((8, 2, 2, KR, 128), bf16),
            pltpu.VMEM((2, 7, NH, 256), f32),
            pltpu.VMEM((8, 2, 8, 256), f32),
            pltpu.SMEM((1,), jnp.int32),
            pltpu.SemaphoreType.DMA((7 + NP + 3,)),
            pltpu.SemaphoreType.DMA((NP,)),
            pltpu.SemaphoreType.DMA((7,)),
        ],
        compiler_params=pltpu.CompilerParams(
            vmem_limit_bytes=120 * 1024 * 1024,
            disable_bounds_checks=True,
            disable_semaphore_checks=True),
    )(jnp.transpose(x, (1, 2, 0)), w, g, b)
    return jnp.transpose(out, (2, 0, 1))
```

```python
import functools
import itertools

import jax
import jax.numpy as jnp
from jax import lax
import jax.experimental.pallas as pl
import jax.experimental.pallas.tpu as pltpu

f32 = jnp.float32
bf16 = jnp.bfloat16
u32 = jnp.uint32

S, D, B = 32, 576, 1024
KH = 256
NH, NQ = 288, 144
KR = 80
NP = S // 2
EPS = 1e-5

SWAP = (False, True, False, False, True, True, True)

STATS_OPS, NORM_OPS, REM_OPS = 710, 255, 112
UNIT_OPS = 2 * STATS_OPS + 8 * NORM_OPS + REM_OPS


def _as_bf16(v):
    return pltpu.bitcast(v, bf16)


def _dot(a, b):
    return jnp.dot(a, b, preferred_element_type=f32)


def _add(x, y):
    return x + y


def _sub(x, y):
    return x - y


def _add2(a, b):
    return [[a[i][j] + b[i][j] for j in range(2)] for i in range(2)]


def _sub2(a, b):
    return [[a[i][j] - b[i][j] for j in range(2)] for i in range(2)]


def _strassen_lhs(a, add, sub):
    (a11, a12), (a21, a22) = a
    return [add(a11, a22), add(a21, a22), a11, a22, add(a11, a12), sub(a21, a11), sub(a12, a22)]


def _prepare_weights(w_ref, g_ref, b_ref, af_ref, as_ref, ar_ref):
    g_row = g_ref[...].astype(f32).reshape(1, D)
    b_row = b_ref[...].astype(f32).reshape(1, D)
    w = w_ref[...]
    rid = lax.broadcasted_iota(jnp.int32, (16, D), 0)
    bmat = jnp.where(rid < 2, jnp.broadcast_to(b_row, (16, D)), 0.0).astype(bf16)
    bias = _dot(bmat, w)
    hi = bias.astype(bf16).astype(f32)
    extra = jnp.where(rid == 0, hi, bias - hi)
    waug = jnp.concatenate([w.astype(f32), extra, jnp.zeros((48, D), f32)], axis=0)
    waug = jnp.concatenate([waug, jnp.zeros((640, 64), f32)], axis=1)
    gaug = jnp.concatenate([g_row, jnp.ones((1, 64), f32)], axis=1)
    a = waug.T[:D] * gaug
    for kt in range(4):
        af_ref[kt] = a[:, 128 * kt:128 * (kt + 1)]
    ar_ref[...] = a[:, 2 * KH:].astype(bf16)
    for q in range(NQ // 16):
        def blk(i2, k2):
            return [[af_ref[2 * k2 + k, pl.ds(NQ * (2 * i2 + i) + 16 * q, 16), :] for k in range(2)]
                    for i in range(2)]
        outer = _strassen_lhs([[blk(0, 0), blk(0, 1)], [blk(1, 0), blk(1, 1)]], _add2, _sub2)
        for o in range(7):
            for n, v in enumerate(_strassen_lhs(outer[o], _add, _sub)):
                as_ref[7 * o + n, 16 * q:16 * q + 16, :] = v.astype(bf16)


MAIN_KNOBS = dict(lead=200, trail=0, wrem=0.95, wfin=0.58)
HEAD_KNOBS = (
    dict(lead=30, trail=-300, wrem=1.09, wfin=0.55),
    dict(lead=200, trail=-50, wrem=0.92, wfin=0.57),
    dict(lead=30, trail=-50, wrem=1.08, wfin=0.68),
    dict(lead=30, trail=-250, wrem=0.97, wfin=0.51),
    dict(lead=30, trail=-300, wrem=1.09, wfin=0.55),
)
HEAD_PLAN = (1.0, 1.5, 1.5, 3.0, 4.0)
RC = 48
WRITE_FROM = 7
WCOLS = 128
BCOLS = 256


def _kernel(x_hbm, w_hbm, g_hbm, b_hbm, o_hbm,
            xbuf, obuf, wbuf, g_ref, b_ref, af_ref, as_ref, ar_ref, bs, br, tb, sb, flag,
            isem, osem, tsem):
    as_u, ar_u, bs_u, br_u = (r.bitcast(u32) for r in (as_ref, ar_ref, bs, br))

    chunks = [(0, 0, 256), (0, 256, 256), (0, 512, 512), (2, 0, 512), (2, 512, 512),
              (4, 0, 512), (4, 512, 512)]
    nch = len(chunks)

    def read_chunk(i):
        s0, c0, nc = chunks[i]
        sl = (pl.ds(s0, 2), slice(None), pl.ds(c0, nc))
        return pltpu.make_async_copy(x_hbm.at[sl], xbuf.at[sl], isem.at[i])

    def read_pair(p):
        return pltpu.make_async_copy(x_hbm.at[pl.ds(2 * p, 2)], xbuf.at[pl.ds(2 * p, 2)], isem.at[nch + p])

    def write_slices(s0, ns, k, wc=WCOLS):
        sls = [(pl.ds(s0, ns), slice(None), pl.ds(c, wc)) for c in range(0, B, wc)]
        return [pltpu.make_async_copy(obuf.at[sl], o_hbm.at[sl], osem.at[k]) for sl in sls]

    param_copies = [pltpu.make_async_copy(src, dst, isem.at[nch + NP + i])
                    for i, (src, dst) in enumerate(((w_hbm, wbuf), (g_hbm, g_ref), (b_hbm, b_ref)))]
    for c in param_copies:
        c.start()
    for i in range(nch):
        read_chunk(i).start()
    for p in range(3, NP):
        read_pair(p).start()

    flag[0] = 1
    rid = lax.broadcasted_iota(jnp.int32, (KR - 64, 128), 0)
    ones = (rid < 2).astype(f32).astype(bf16)
    for t in range(8):
        for j in range(2):
            for h in range(2):
                br[t, j, h, 64:KR, :] = ones
    for c in param_copies:
        c.wait()
    _prepare_weights(wbuf, g_ref, b_ref, af_ref, as_ref, ar_ref)

    def stats_item(sl, g, slot, j):
        cols = slice(256 * g, 256 * g + 256)
        ld = lambda q: xbuf[sl[j], 8 * q:8 * q + 8, cols].astype(f32)
        nb = D // 8
        c = ld(0)
        s1 = s2 = None
        for q in range(1, nb):
            d = ld(q) - c
            s1 = d if s1 is None else s1 + d
            s2 = d * d if s2 is None else s2 + d * d
            yield 10
        dm = s1 * (1.0 / nb)
        mj = c + dm
        m = jnp.sum(mj, axis=0, keepdims=True) * 0.125
        e = mj - m
        m2 = (s2 - s1 * dm) + (e * e) * float(nb)
        var = jnp.maximum(jnp.sum(m2, axis=0, keepdims=True) * (1.0 / D), 0.0)
        sb[slot, j, 0:1, :] = m
        sb[slot, j, 1:2, :] = lax.rsqrt(var + EPS)

    def norm_item(sl, g, slot, q):
        cols = slice(256 * g, 256 * g + 256)

        def nrm(j, r0):
            return (xbuf[sl[j], r0:r0 + 16, cols].astype(f32) - sb[slot, j, 0:1, :]) * sb[slot, j, 1:2, :]

        if q == 8:
            for j in range(2):
                for r in range(0, 64, 16):
                    v = nrm(j, 2 * KH + r)
                    br[slot, j, 0, r:r + 16, :] = v[:, :128].astype(bf16)
                    br[slot, j, 1, r:r + 16, :] = v[:, 128:].astype(bf16)
                    yield 14
            return

        def blk(k2, j):
            return [[v[:, :128], v[:, 128:]] for v in (nrm(j, KH * k2 + 128 * k + 16 * q) for k in range(2))]

        def emit(o, b):
            (b11, b12), (b21, b22) = [row[::-1] for row in b] if SWAP[o] else b

            def put(n, v):
                bs[slot, 7 * o + n, 16 * q:16 * q + 16, :] = v.astype(bf16)

            put(0, b11 + b22)
            put(1, b11)
            put(2, b12 - b22)
            put(3, b21 - b11)
            yield 10
            put(4, b22)
            put(5, b11 + b12)
            put(6, b21 + b22)
            yield 7

        def emit_sum(o, comb, x, y):
            t = comb(x, y)
            yield 8
            yield from emit(o, t)

        b11 = blk(0, 0)
        yield 24
        yield from emit(1, b11)
        b12 = blk(0, 1)
        yield 24
        yield from emit_sum(5, _add2, b11, b12)
        b22 = blk(1, 1)
        yield 24
        yield from emit_sum(2, _sub2, b12, b22)
        yield from emit_sum(0, _add2, b11, b22)
        yield from emit(4, b22)
        b21 = blk(1, 0)
        yield 24
        yield from emit_sum(3, _sub2, b21, b11)
        yield from emit_sum(6, _add2, b21, b22)

    class LnQueue:
        def __init__(self, units):
            self.stats = [(u, (sl, g, slot, j), STATS_OPS)
                          for u, (sl, g, slot) in enumerate(units) for j in range(2)]
            self.norm = [(u, (sl, g, slot, q), NORM_OPS if q < 8 else REM_OPS)
                         for u, (sl, g, slot) in enumerate(units) for q in range(9)]

        def take(self, budget, max_unit, need):
            st, nm = self.stats, self.norm
            slack = budget - sum(it[2] for it in st + nm if it[0] <= need)
            left = lambda items, u: sum(it[2] for it in items if it[0] == u)
            seq = []
            while True:
                ok = lambda it: it[0] <= need or (it[0] <= max_unit and slack >= it[2])
                s_ok = bool(st) and ok(st[0]) and not (nm and st[0][0] > nm[0][0] + 1)
                n_ok = bool(nm) and ok(nm[0]) and not (st and st[0][0] <= nm[0][0])
                if not (s_ok or n_ok):
                    break
                if s_ok and n_ok:
                    u = nm[0][0]
                    s_ok = left(st, u + 1) / (2 * STATS_OPS) >= left(nm, u) / (8 * NORM_OPS + REM_OPS)
                it = (st if s_ok else nm).pop(0)
                if it[0] > need:
                    slack -= it[2]
                seq.append((s_ok, it))
            assert not any(it[0] <= need for it in st + nm)

            def gen():
                i = 0
                while i < len(seq):
                    is_stats, it = seq[i]
                    i += 1
                    if not is_stats:
                        yield from norm_item(*it[1])
                        continue
                    follow = []
                    while i < len(seq) and not seq[i][0] and seq[i][1][0] < it[0]:
                        follow.append(seq[i][1])
                        i += 1
                    ng = itertools.chain.from_iterable(norm_item(*f[1]) for f in follow)
                    ntot = sum(f[2] for f in follow)
                    ds = dn = 0
                    for n in stats_item(*it[1]):
                        ds += n
                        yield n
                        while dn * it[2] < ds * ntot:
                            m = next(ng, None)
                            if m is None:
                                break
                            dn += m
                            yield m
                    yield from ng

            return gen, sum(it[2] for _, it in seq)

    def mm_unit(unit, tp, tick, done, kn):
        sl, g, slot = unit
        cols = slice(256 * g, 256 * g + 256)
        wtot = 35 + 14 * kn['wfin'] + 16 * kn['wrem']

        def prod(o, post):
            w = RC / NQ / wtot * (kn['wfin'] if o >= 5 else 1.0)
            for r0 in range(0, NQ, RC):
                p = {}
                for n in (5, 3, 1, 7, 4, 2, 6):
                    if p:
                        tick(w)
                    p[n] = _dot(_as_bf16(as_u[7 * o + n - 1, r0 // 2:(r0 + RC) // 2, :]),
                                _as_bf16(bs_u[slot, 7 * o + n - 1]))
                t12 = p[5] + p[3]
                t11 = ((p[1] + p[7]) - p[5]) + p[4]
                t22 = (p[1] + p[3]) + (p[6] - p[2])
                t21 = p[2] + p[4]
                if SWAP[o]:
                    t11, t12, t21, t22 = t12, t11, t22, t21
                top, bot = jnp.concatenate([t11, t12], axis=1), jnp.concatenate([t21, t22], axis=1)
                post(slice(r0, r0 + RC), top)
                post(slice(NQ + r0, NQ + r0 + RC), bot)
                tick(w)

        def rem(i2, j, post):
            for r0 in range(0, NH, RC):
                v = _dot(_as_bf16(ar_u[(NH * i2 + r0) // 2:(NH * i2 + r0 + RC) // 2, :])[:, :KR],
                         jnp.concatenate([_as_bf16(br_u[slot, j, 0]), _as_bf16(br_u[slot, j, 1])], axis=1))
                post(slice(r0, r0 + RC), v)
                tick(kn['wrem'] * 2 * RC / NQ / wtot)

        def ld(k, r):
            return tb[tp, k, r, :]

        def keep(k):
            def post(r, v):
                tb[tp, k, r, :] = v
            return post

        def out(i2, j, r, v):
            obuf[sl[j], NH * i2 + r.start:NH * i2 + r.stop, cols] = v.astype(bf16)

        prod(1, keep(1))
        prod(3, keep(3))
        rem(1, 0, lambda r, v: out(1, 0, r, v + (ld(1, r) + ld(3, r))))
        done(1, 0)
        prod(2, keep(2))
        prod(4, keep(4))
        rem(0, 1, lambda r, v: out(0, 1, r, v + (ld(2, r) + ld(4, r))))
        done(0, 1)
        prod(0, keep(0))
        rem(0, 0, lambda r, v: keep(5)(r, (v + ld(0, r)) + (ld(3, r) - ld(4, r))))
        prod(6, lambda r, v: out(0, 0, r, v + ld(5, r)))
        done(0, 0)
        rem(1, 1, lambda r, v: keep(6)(r, (v + ld(0, r)) + (ld(2, r) - ld(1, r))))
        prod(5, lambda r, v: out(1, 1, r, v + ld(6, r)))
        done(1, 1)

    def phase(units, make_ln_gen, ln_ops, kn, done=lambda u, i2, j: None):
        ln_gen = make_ln_gen()
        quota = max(ln_ops - kn['lead'] - kn['trail'], 0) / len(units)
        debt = [0.0]

        def pay(n):
            debt[0] += n
            while debt[0] > 0:
                step = next(ln_gen, None)
                if step is None:
                    return
                debt[0] -= step

        pay(kn['lead'])
        for i, u in enumerate(units):
            mm_unit(u, i % 2, lambda w: pay(quota * w), functools.partial(done, i), kn)
        for _ in ln_gen:
            pass

    hu = [([2 * (u // 4), 2 * (u // 4) + 1], u % 4, u % 8) for u in range(12)]
    ln = LnQueue(hu)
    read_chunk(0).wait()

    first_stats = [ln.stats.pop(0) for _ in range(2)]
    first_norm = [ln.norm.pop(0) for _ in range(9)]

    @pl.when(flag[0] == 1)
    def _():
        for _ in itertools.zip_longest(*[stats_item(*it[1]) for it in first_stats]):
            pass

    @pl.when(flag[0] == 1)
    def _():
        for it in first_norm:
            for _ in norm_item(*it[1]):
                pass

    head = [(hu[0:1], 1, 1, (1,)), (hu[1:2], 3, 2, (2,)), (hu[2:3], 5, 4, (3,)),
            (hu[3:5], 7, 7, (4,)), (hu[5:8], 11, 11, (5, 6))]
    for k, (units, max_unit, need, waits) in enumerate(head):
        for i in waits:
            read_chunk(i).wait()
        gen, ops = ln.take(HEAD_PLAN[k] * UNIT_OPS, max_unit, need)
        pl.when(flag[0] == 1)(functools.partial(phase, units, gen, ops, HEAD_KNOBS[k]))

    def body(p, carry):
        cur = [2 * p, 2 * p + 1]
        nxt = [jnp.minimum(2 * p + 2, S - 1), jnp.minimum(2 * p + 3, S - 1)]
        read_pair(p + 1).wait()

        for par in range(2):
            @pl.when((p & 1) == par)
            def _():
                gen, ops = LnQueue([(nxt, g, 4 * (1 - par) + g) for g in range(4)]).take(0, 3, 3)
                phase([(cur, g, 4 * par + g) for g in range(4)], gen, ops, MAIN_KNOBS)
                if par == (WRITE_FROM - 1) % 2:
                    @pl.when(p == WRITE_FROM - 1)
                    def _():
                        for c in write_slices(0, 2 * WRITE_FROM, 0, BCOLS):
                            c.start()

                @pl.when(p >= WRITE_FROM)
                def _():
                    for c in write_slices(2 * p, 2, p):
                        c.start()
        return carry

    lax.fori_loop(2, NP - 1, body, 0)

    tail = []

    def send(sl):
        c = pltpu.make_async_copy(obuf.at[sl], o_hbm.at[sl], tsem.at[len(tail)])
        c.start()
        tail.append(c)

    def done_last(u, i2, j):
        cols = pl.ds(256 * u, 256)
        if u == 3:
            send((S - 2 + j, pl.ds(NH * i2, NH), cols))
        elif (i2, j) == (1, 1):
            send((pl.ds(S - 2, 2), slice(None), cols))

    phase([([S - 2, S - 1], g, 4 + g) for g in range(4)], lambda: iter(()), 0, MAIN_KNOBS, done_last)

    for c in write_slices(0, 2 * WRITE_FROM, 0, BCOLS):
        c.wait()
    for p in range(WRITE_FROM, NP - 1):
        for c in write_slices(2 * p, 2, p):
            c.wait()
    for c in tail:
        c.wait()


@jax.jit
def pallas_standalone__layernorm_linear__sampling_kernel(
    x: jax.Array,
    g: jax.Array,
    b: jax.Array,
    w: jax.Array,
):
    assert x.shape == (B, S, D) and w.shape == (D, D)
    out = pl.pallas_call(
        _kernel,
        in_specs=[pl.BlockSpec(memory_space=pl.ANY)] * 4,
        out_specs=pl.BlockSpec(memory_space=pl.ANY),
        out_shape=jax.ShapeDtypeStruct((S, D, B), x.dtype),
        scratch_shapes=[
            pltpu.VMEM((S, D, B), bf16),
            pltpu.VMEM((S, D, B), bf16),
            pltpu.VMEM((D, D), bf16),
            pltpu.VMEM((D,), bf16),
            pltpu.VMEM((D,), bf16),
            pltpu.VMEM((4, D, 128), f32),
            pltpu.VMEM((49, NQ, 128), bf16),
            pltpu.VMEM((D, 128), bf16),
            pltpu.VMEM((8, 49, 128, 128), bf16),
            pltpu.VMEM((8, 2, 2, KR, 128), bf16),
            pltpu.VMEM((2, 7, NH, 256), f32),
            pltpu.VMEM((8, 2, 8, 256), f32),
            pltpu.SMEM((1,), jnp.int32),
            pltpu.SemaphoreType.DMA((7 + NP + 3,)),
            pltpu.SemaphoreType.DMA((NP,)),
            pltpu.SemaphoreType.DMA((7,)),
        ],
        compiler_params=pltpu.CompilerParams(
            vmem_limit_bytes=120 * 1024 * 1024,
            disable_bounds_checks=True,
            disable_semaphore_checks=True),
    )(jnp.transpose(x, (1, 2, 0)), w, g, b)
    return jnp.transpose(out, (2, 0, 1))
```

```python
import functools
import itertools

import jax
import jax.numpy as jnp
from jax import lax
import jax.experimental.pallas as pl
import jax.experimental.pallas.tpu as pltpu

f32 = jnp.float32
bf16 = jnp.bfloat16
u32 = jnp.uint32

S, D, B = 32, 576, 1024
KH = 256
NH, NQ = 288, 144
KR = 80
NP = S // 2
EPS = 1e-5

SWAP = (False, True, False, False, True, True, True)

STATS_OPS, NORM_OPS, REM_OPS = 710, 255, 112
UNIT_OPS = 2 * STATS_OPS + 8 * NORM_OPS + REM_OPS


def _as_bf16(v):
    return pltpu.bitcast(v, bf16)


def _dot(a, b):
    return jnp.dot(a, b, preferred_element_type=f32)


def _add(x, y):
    return x + y


def _sub(x, y):
    return x - y


def _add2(a, b):
    return [[a[i][j] + b[i][j] for j in range(2)] for i in range(2)]


def _sub2(a, b):
    return [[a[i][j] - b[i][j] for j in range(2)] for i in range(2)]


def _strassen_lhs(a, add, sub):
    (a11, a12), (a21, a22) = a
    return [add(a11, a22), add(a21, a22), a11, a22, add(a11, a12), sub(a21, a11), sub(a12, a22)]


def _prepare_weights(w_ref, g_ref, b_ref, af_ref, as_ref, ar_ref):
    g_row = g_ref[...].astype(f32).reshape(1, D)
    b_row = b_ref[...].astype(f32).reshape(1, D)
    w = w_ref[...]
    rid = lax.broadcasted_iota(jnp.int32, (16, D), 0)
    bmat = jnp.where(rid < 2, jnp.broadcast_to(b_row, (16, D)), 0.0).astype(bf16)
    bias = _dot(bmat, w)
    hi = bias.astype(bf16).astype(f32)
    extra = jnp.where(rid == 0, hi, bias - hi)
    waug = jnp.concatenate([w.astype(f32), extra, jnp.zeros((48, D), f32)], axis=0)
    waug = jnp.concatenate([waug, jnp.zeros((640, 64), f32)], axis=1)
    gaug = jnp.concatenate([g_row, jnp.ones((1, 64), f32)], axis=1)
    a = waug.T[:D] * gaug
    for kt in range(4):
        af_ref[kt] = a[:, 128 * kt:128 * (kt + 1)]
    ar_ref[...] = a[:, 2 * KH:].astype(bf16)
    for q in range(NQ // 16):
        def blk(i2, k2):
            return [[af_ref[2 * k2 + k, pl.ds(NQ * (2 * i2 + i) + 16 * q, 16), :] for k in range(2)]
                    for i in range(2)]
        outer = _strassen_lhs([[blk(0, 0), blk(0, 1)], [blk(1, 0), blk(1, 1)]], _add2, _sub2)
        for o in range(7):
            for n, v in enumerate(_strassen_lhs(outer[o], _add, _sub)):
                as_ref[7 * o + n, 16 * q:16 * q + 16, :] = v.astype(bf16)


_ROWS2 = ((0, 80), (80, 64))
_ROWS3 = ((0, 48), (48, 48), (96, 48))
MAIN_KNOBS = dict(lead=30, trail=0, wrem=1.33, wfin=0.52, rows=_ROWS2)
HEAD_KNOBS = (
    dict(lead=30, trail=-300, wrem=1.09, wfin=0.55, rows=_ROWS3),
    dict(lead=200, trail=-50, wrem=0.92, wfin=0.57, rows=_ROWS3),
    dict(lead=30, trail=-50, wrem=1.08, wfin=0.68, rows=_ROWS3),
    dict(lead=30, trail=-250, wrem=0.97, wfin=0.51, rows=_ROWS3),
    dict(lead=30, trail=-300, wrem=1.09, wfin=0.55, rows=_ROWS3),
)
HEAD_PLAN = (1.0, 1.5, 1.5, 3.0, 4.0)
RC = 48
WRITE_FROM = 7
WCOLS = 128
BCOLS = 256


def _kernel(x_hbm, w_hbm, g_hbm, b_hbm, o_hbm,
            xbuf, obuf, wbuf, g_ref, b_ref, af_ref, as_ref, ar_ref, bs, br, tb, sb, flag,
            isem, osem, tsem):
    as_u, ar_u, bs_u, br_u = (r.bitcast(u32) for r in (as_ref, ar_ref, bs, br))

    chunks = [(0, 0, 256), (0, 256, 256), (0, 512, 512), (2, 0, 512), (2, 512, 512),
              (4, 0, 512), (4, 512, 512)]
    nch = len(chunks)

    def read_chunk(i):
        s0, c0, nc = chunks[i]
        sl = (pl.ds(s0, 2), slice(None), pl.ds(c0, nc))
        return pltpu.make_async_copy(x_hbm.at[sl], xbuf.at[sl], isem.at[i])

    def read_pair(p):
        return pltpu.make_async_copy(x_hbm.at[pl.ds(2 * p, 2)], xbuf.at[pl.ds(2 * p, 2)], isem.at[nch + p])

    def write_slices(s0, ns, k, wc=WCOLS):
        sls = [(pl.ds(s0, ns), slice(None), pl.ds(c, wc)) for c in range(0, B, wc)]
        return [pltpu.make_async_copy(obuf.at[sl], o_hbm.at[sl], osem.at[k]) for sl in sls]

    param_copies = [pltpu.make_async_copy(src, dst, isem.at[nch + NP + i])
                    for i, (src, dst) in enumerate(((w_hbm, wbuf), (g_hbm, g_ref), (b_hbm, b_ref)))]
    for c in param_copies:
        c.start()
    for i in range(nch):
        read_chunk(i).start()
    for p in range(3, NP):
        read_pair(p).start()

    flag[0] = 1
    rid = lax.broadcasted_iota(jnp.int32, (KR - 64, 128), 0)
    ones = (rid < 2).astype(f32).astype(bf16)
    for t in range(8):
        for j in range(2):
            for h in range(2):
                br[t, j, h, 64:KR, :] = ones
    for c in param_copies:
        c.wait()
    _prepare_weights(wbuf, g_ref, b_ref, af_ref, as_ref, ar_ref)

    def stats_item(sl, g, slot, j):
        cols = slice(256 * g, 256 * g + 256)
        ld = lambda q: xbuf[sl[j], 8 * q:8 * q + 8, cols].astype(f32)
        nb = D // 8
        c = ld(0)
        s1 = s2 = None
        for q in range(1, nb):
            d = ld(q) - c
            s1 = d if s1 is None else s1 + d
            s2 = d * d if s2 is None else s2 + d * d
            yield 10
        dm = s1 * (1.0 / nb)
        mj = c + dm
        m = jnp.sum(mj, axis=0, keepdims=True) * 0.125
        e = mj - m
        m2 = (s2 - s1 * dm) + (e * e) * float(nb)
        var = jnp.maximum(jnp.sum(m2, axis=0, keepdims=True) * (1.0 / D), 0.0)
        sb[slot, j, 0:1, :] = m
        sb[slot, j, 1:2, :] = lax.rsqrt(var + EPS)

    def norm_item(sl, g, slot, q):
        cols = slice(256 * g, 256 * g + 256)

        def nrm(j, r0):
            return (xbuf[sl[j], r0:r0 + 16, cols].astype(f32) - sb[slot, j, 0:1, :]) * sb[slot, j, 1:2, :]

        if q == 8:
            for j in range(2):
                for r in range(0, 64, 16):
                    v = nrm(j, 2 * KH + r)
                    br[slot, j, 0, r:r + 16, :] = v[:, :128].astype(bf16)
                    br[slot, j, 1, r:r + 16, :] = v[:, 128:].astype(bf16)
                    yield 14
            return

        def blk(k2, j):
            return [[v[:, :128], v[:, 128:]] for v in (nrm(j, KH * k2 + 128 * k + 16 * q) for k in range(2))]

        def emit(o, b):
            (b11, b12), (b21, b22) = [row[::-1] for row in b] if SWAP[o] else b

            def put(n, v):
                bs[slot, 7 * o + n, 16 * q:16 * q + 16, :] = v.astype(bf16)

            put(0, b11 + b22)
            put(1, b11)
            put(2, b12 - b22)
            put(3, b21 - b11)
            yield 10
            put(4, b22)
            put(5, b11 + b12)
            put(6, b21 + b22)
            yield 7

        def emit_sum(o, comb, x, y):
            t = comb(x, y)
            yield 8
            yield from emit(o, t)

        b11 = blk(0, 0)
        yield 24
        yield from emit(1, b11)
        b12 = blk(0, 1)
        yield 24
        yield from emit_sum(5, _add2, b11, b12)
        b22 = blk(1, 1)
        yield 24
        yield from emit_sum(2, _sub2, b12, b22)
        yield from emit_sum(0, _add2, b11, b22)
        yield from emit(4, b22)
        b21 = blk(1, 0)
        yield 24
        yield from emit_sum(3, _sub2, b21, b11)
        yield from emit_sum(6, _add2, b21, b22)

    class LnQueue:
        def __init__(self, units):
            self.stats = [(u, (sl, g, slot, j), STATS_OPS)
                          for u, (sl, g, slot) in enumerate(units) for j in range(2)]
            self.norm = [(u, (sl, g, slot, q), NORM_OPS if q < 8 else REM_OPS)
                         for u, (sl, g, slot) in enumerate(units) for q in range(9)]

        def take(self, budget, max_unit, need):
            st, nm = self.stats, self.norm
            slack = budget - sum(it[2] for it in st + nm if it[0] <= need)
            left = lambda items, u: sum(it[2] for it in items if it[0] == u)
            seq = []
            while True:
                ok = lambda it: it[0] <= need or (it[0] <= max_unit and slack >= it[2])
                s_ok = bool(st) and ok(st[0]) and not (nm and st[0][0] > nm[0][0] + 1)
                n_ok = bool(nm) and ok(nm[0]) and not (st and st[0][0] <= nm[0][0])
                if not (s_ok or n_ok):
                    break
                if s_ok and n_ok:
                    u = nm[0][0]
                    s_ok = left(st, u + 1) / (2 * STATS_OPS) >= left(nm, u) / (8 * NORM_OPS + REM_OPS)
                it = (st if s_ok else nm).pop(0)
                if it[0] > need:
                    slack -= it[2]
                seq.append((s_ok, it))
            assert not any(it[0] <= need for it in st + nm)

            def gen():
                i = 0
                while i < len(seq):
                    is_stats, it = seq[i]
                    i += 1
                    if not is_stats:
                        yield from norm_item(*it[1])
                        continue
                    follow = []
                    while i < len(seq) and not seq[i][0] and seq[i][1][0] < it[0]:
                        follow.append(seq[i][1])
                        i += 1
                    ng = itertools.chain.from_iterable(norm_item(*f[1]) for f in follow)
                    ntot = sum(f[2] for f in follow)
                    ds = dn = 0
                    for n in stats_item(*it[1]):
                        ds += n
                        yield n
                        while dn * it[2] < ds * ntot:
                            m = next(ng, None)
                            if m is None:
                                break
                            dn += m
                            yield m
                    yield from ng

            return gen, sum(it[2] for _, it in seq)

    def mm_unit(unit, tp, tick, done, kn):
        sl, g, slot = unit
        cols = slice(256 * g, 256 * g + 256)
        wtot = 35 + 14 * kn['wfin'] + 16 * kn['wrem']

        def prod(o, post):
            for r0, rc in kn['rows']:
                w = rc / NQ / wtot * (kn['wfin'] if o >= 5 else 1.0)
                p = {}
                for n in (5, 3, 1, 7, 4, 2, 6):
                    if p:
                        tick(w)
                    p[n] = _dot(_as_bf16(as_u[7 * o + n - 1, r0 // 2:(r0 + rc) // 2, :]),
                                _as_bf16(bs_u[slot, 7 * o + n - 1]))
                t12 = p[5] + p[3]
                t11 = ((p[1] + p[7]) - p[5]) + p[4]
                t22 = (p[1] + p[3]) + (p[6] - p[2])
                t21 = p[2] + p[4]
                if SWAP[o]:
                    t11, t12, t21, t22 = t12, t11, t22, t21
                top, bot = jnp.concatenate([t11, t12], axis=1), jnp.concatenate([t21, t22], axis=1)
                post(slice(r0, r0 + rc), top)
                post(slice(NQ + r0, NQ + r0 + rc), bot)
                tick(w)

        def rem(i2, j, post):
            for r0 in range(0, NH, RC):
                v = _dot(_as_bf16(ar_u[(NH * i2 + r0) // 2:(NH * i2 + r0 + RC) // 2, :])[:, :KR],
                         jnp.concatenate([_as_bf16(br_u[slot, j, 0]), _as_bf16(br_u[slot, j, 1])], axis=1))
                post(slice(r0, r0 + RC), v)
                tick(kn['wrem'] * 2 * RC / NQ / wtot)

        def ld(k, r):
            return tb[tp, k, r, :]

        def keep(k):
            def post(r, v):
                tb[tp, k, r, :] = v
            return post

        def out(i2, j, r, v):
            obuf[sl[j], NH * i2 + r.start:NH * i2 + r.stop, cols] = v.astype(bf16)

        prod(1, keep(1))
        prod(3, keep(3))
        rem(1, 0, lambda r, v: out(1, 0, r, v + (ld(1, r) + ld(3, r))))
        done(1, 0)
        prod(2, keep(2))
        prod(4, keep(4))
        rem(0, 1, lambda r, v: out(0, 1, r, v + (ld(2, r) + ld(4, r))))
        done(0, 1)
        prod(0, keep(0))
        rem(0, 0, lambda r, v: keep(5)(r, (v + ld(0, r)) + (ld(3, r) - ld(4, r))))
        prod(6, lambda r, v: out(0, 0, r, v + ld(5, r)))
        done(0, 0)
        rem(1, 1, lambda r, v: keep(6)(r, (v + ld(0, r)) + (ld(2, r) - ld(1, r))))
        prod(5, lambda r, v: out(1, 1, r, v + ld(6, r)))
        done(1, 1)

    def phase(units, make_ln_gen, ln_ops, kn, done=lambda u, i2, j: None):
        ln_gen = make_ln_gen()
        quota = max(ln_ops - kn['lead'] - kn['trail'], 0) / len(units)
        debt = [0.0]

        def pay(n):
            debt[0] += n
            while debt[0] > 0:
                step = next(ln_gen, None)
                if step is None:
                    return
                debt[0] -= step

        pay(kn['lead'])
        for i, u in enumerate(units):
            mm_unit(u, i % 2, lambda w: pay(quota * w), functools.partial(done, i), kn)
        for _ in ln_gen:
            pass

    hu = [([2 * (u // 4), 2 * (u // 4) + 1], u % 4, u % 8) for u in range(12)]
    ln = LnQueue(hu)
    read_chunk(0).wait()

    first_stats = [ln.stats.pop(0) for _ in range(2)]
    first_norm = [ln.norm.pop(0) for _ in range(9)]

    @pl.when(flag[0] == 1)
    def _():
        for _ in itertools.zip_longest(*[stats_item(*it[1]) for it in first_stats]):
            pass

    @pl.when(flag[0] == 1)
    def _():
        for it in first_norm:
            for _ in norm_item(*it[1]):
                pass

    head = [(hu[0:1], 1, 1, (1,)), (hu[1:2], 3, 2, (2,)), (hu[2:3], 5, 4, (3,)),
            (hu[3:5], 7, 7, (4,)), (hu[5:8], 11, 11, (5, 6))]
    for k, (units, max_unit, need, waits) in enumerate(head):
        for i in waits:
            read_chunk(i).wait()
        gen, ops = ln.take(HEAD_PLAN[k] * UNIT_OPS, max_unit, need)
        pl.when(flag[0] == 1)(functools.partial(phase, units, gen, ops, HEAD_KNOBS[k]))

    def body(p, carry):
        cur = [2 * p, 2 * p + 1]
        nxt = [jnp.minimum(2 * p + 2, S - 1), jnp.minimum(2 * p + 3, S - 1)]
        read_pair(p + 1).wait()

        for par in range(2):
            @pl.when((p & 1) == par)
            def _():
                gen, ops = LnQueue([(nxt, g, 4 * (1 - par) + g) for g in range(4)]).take(0, 3, 3)
                phase([(cur, g, 4 * par + g) for g in range(4)], gen, ops, MAIN_KNOBS)
                if par == (WRITE_FROM - 1) % 2:
                    @pl.when(p == WRITE_FROM - 1)
                    def _():
                        for c in write_slices(0, 2 * WRITE_FROM, 0, BCOLS):
                            c.start()

                @pl.when(p >= WRITE_FROM)
                def _():
                    for c in write_slices(2 * p, 2, p):
                        c.start()
        return carry

    lax.fori_loop(2, NP - 1, body, 0)

    tail = []

    def send(sl):
        c = pltpu.make_async_copy(obuf.at[sl], o_hbm.at[sl], tsem.at[len(tail)])
        c.start()
        tail.append(c)

    def done_last(u, i2, j):
        cols = pl.ds(256 * u, 256)
        if u == 3:
            send((S - 2 + j, pl.ds(NH * i2, NH), cols))
        elif (i2, j) == (1, 1):
            send((pl.ds(S - 2, 2), slice(None), cols))

    phase([([S - 2, S - 1], g, 4 + g) for g in range(4)], lambda: iter(()), 0, MAIN_KNOBS, done_last)

    for c in write_slices(0, 2 * WRITE_FROM, 0, BCOLS):
        c.wait()
    for p in range(WRITE_FROM, NP - 1):
        for c in write_slices(2 * p, 2, p):
            c.wait()
    for c in tail:
        c.wait()


@jax.jit
def pallas_standalone__layernorm_linear__sampling_kernel(
    x: jax.Array,
    g: jax.Array,
    b: jax.Array,
    w: jax.Array,
):
    assert x.shape == (B, S, D) and w.shape == (D, D)
    out = pl.pallas_call(
        _kernel,
        in_specs=[pl.BlockSpec(memory_space=pl.ANY)] * 4,
        out_specs=pl.BlockSpec(memory_space=pl.ANY),
        out_shape=jax.ShapeDtypeStruct((S, D, B), x.dtype),
        scratch_shapes=[
            pltpu.VMEM((S, D, B), bf16),
            pltpu.VMEM((S, D, B), bf16),
            pltpu.VMEM((D, D), bf16),
            pltpu.VMEM((D,), bf16),
            pltpu.VMEM((D,), bf16),
            pltpu.VMEM((4, D, 128), f32),
            pltpu.VMEM((49, NQ, 128), bf16),
            pltpu.VMEM((D, 128), bf16),
            pltpu.VMEM((8, 49, 128, 128), bf16),
            pltpu.VMEM((8, 2, 2, KR, 128), bf16),
            pltpu.VMEM((2, 7, NH, 256), f32),
            pltpu.VMEM((8, 2, 8, 256), f32),
            pltpu.SMEM((1,), jnp.int32),
            pltpu.SemaphoreType.DMA((7 + NP + 3,)),
            pltpu.SemaphoreType.DMA((NP,)),
            pltpu.SemaphoreType.DMA((7,)),
        ],
        compiler_params=pltpu.CompilerParams(
            vmem_limit_bytes=120 * 1024 * 1024,
            disable_bounds_checks=True,
            disable_semaphore_checks=True),
    )(jnp.transpose(x, (1, 2, 0)), w, g, b)
    return jnp.transpose(out, (2, 0, 1))
```
